```python
import jax
import jax.numpy as jnp

def _softmax(x, axis=-1):
    return jax.nn.softmax(x, axis=axis)
def _gelu(x):
    return jax.nn.gelu(x, approximate=True)
def _silu(x):
    return jax.nn.silu(x)
def _sigmoid(x):
    return jax.nn.sigmoid(x)
def _layernorm(x, axis=-1, eps=1e-5):
    m = jnp.mean(x, axis=axis, keepdims=True)
    v = jnp.var(x, axis=axis, keepdims=True)
    return (x - m) / jnp.sqrt(v + eps)
def _scatter_add(tgt, idx, src, axis=0):
    return tgt.at[idx].add(src)
def _segment_sum(src, seg, n):
    return jax.ops.segment_sum(src, seg, n)
class _Rng:
    def __init__(self, key):
        self._k = key
    def _next(self):
        self._k, sub = jax.random.split(self._k)
        return sub
    def normal(self, shape):
        return jax.random.normal(self._next(), shape, dtype=jnp.bfloat16)
    def randint(self, lo, hi, shape):
        return jax.random.randint(self._next(), shape, lo, hi, dtype=jnp.int32)
    def uniform(self, shape, lo=0.0, hi=1.0):
        return jax.random.uniform(self._next(), shape, jnp.bfloat16, lo, hi)
    def permutation(self, n):
        return jax.random.permutation(self._next(), n)


kernel_name = 'gated_mix__compressed_kv_cla__sliding_local_dilated__prompt'

def setup_inputs():
    _rng = _Rng(jax.random.key(int.from_bytes(__import__("os").urandom(4), "little")))
    _w = (lambda a: (lambda t: t.astype(jnp.bfloat16) if jnp.issubdtype(t.dtype, jnp.floating) else t)(jnp.asarray(a)))
    def _A_setup():
        B, H, Sq, Sk, D, M = 1, 32, 2048, 2048, 128, 1024
        Dc = 4 * D
        return {
            "x": _w((lambda *s: _rng.normal(s) * 0.05)(B, Sq, M)),
            "c_kv": _w((lambda *s: _rng.normal(s) * 0.05)(B, Sk, Dc)),
            "w_q": _w((lambda *s: _rng.normal(s) * 0.05)(M, H, D) * (M ** -0.5)),
            "w_uk": _w((lambda *s: _rng.normal(s) * 0.05)(Dc, H, D) * (Dc ** -0.5)),
            "w_uv": _w((lambda *s: _rng.normal(s) * 0.05)(Dc, H, D) * (Dc ** -0.5)),
            "w_o": _w((lambda *s: _rng.normal(s) * 0.05)(H, D, M) * ((H * D) ** -0.5)),
        }
    _A_in = _A_setup()

    def _B_setup():
        B, S, D = 1, 2048, 1024
        return {
            "x": _w((lambda *s: _rng.normal(s) * 0.05)(B, S, D)),
            "wqkv": _w((lambda *s: _rng.normal(s) * 0.05)(D, 3 * D)),
            "wo": _w((lambda *s: _rng.normal(s) * 0.05)(D, D)),
        }
    _B_in = _B_setup()

    return {
        "A_x": _A_in["x"],
        "A_c_kv": _A_in["c_kv"],
        "A_w_q": _A_in["w_q"],
        "A_w_uk": _A_in["w_uk"],
        "A_w_uv": _A_in["w_uv"],
        "A_w_o": _A_in["w_o"],
        "B_x": _B_in["x"],
        "B_wqkv": _B_in["wqkv"],
        "B_wo": _B_in["wo"],
        "gate_w": _w((lambda *s: _rng.normal(s) * 0.05)(1024)),
    }

def reference(A_x, A_c_kv, A_w_q, A_w_uk, A_w_uv, A_w_o, B_x, B_wqkv, B_wo, gate_w):
    def _A_ref(x, c_kv, w_q, w_uk, w_uv, w_o):
        B, Sq, M = x.shape[0], x.shape[1], x.shape[2]
        Sk = c_kv.shape[1]
        H, D = w_q.shape[1], w_q.shape[2]
        q = jnp.einsum("bqm,mhd->bhqd", x, w_q)
        k = jnp.einsum("bkc,chd->bhkd", c_kv, w_uk)
        v = jnp.einsum("bkc,chd->bhkd", c_kv, w_uv)
        scores = jnp.einsum("bhqd,bhkd->bhqk", q, k) * (D ** -0.5)
        off = Sk - Sq
        qi = jnp.arange(Sq)[:, None]
        kj = jnp.arange(Sk)[None, :]
        cmask = kj <= (qi + off)
        scores = jnp.where(cmask[None, None], scores, -1e9)
        p = _softmax(scores, axis=-1)
        ctx = jnp.einsum("bhqk,bhkd->bhqd", p, v)
        return jnp.einsum("bhqd,hdm->bqm", ctx, w_o)

    def _B_ref(x, wqkv, wo):
        B, S, D = x.shape
        H = 32; Dh = D // H
        W, dil = 8, 2
        qkv = (lambda x, *d: x.transpose(*d))((x @ wqkv).reshape(B, S, 3, H, Dh), 2, 0, 3, 1, 4)
        q, k, v = qkv[0], qkv[1], qkv[2]
        scale = Dh ** -0.5
        pos = jnp.arange(S)
        off = jnp.arange(W) * dil
        idx = pos[:, None] - off[None, :]
        mask = idx >= 0
        idx_c = jnp.where(mask, idx, 0).reshape(-1)
        kg = k[:, :, idx_c, :].reshape(B, H, S, W, Dh)
        vg = v[:, :, idx_c, :].reshape(B, H, S, W, Dh)
        logits = jnp.einsum("bhsd,bhswd->bhsw", q, kg) * scale
        logits = jnp.where(mask[None, None, :, :], logits, -1e9)
        attn = _softmax(logits, axis=-1)
        o = jnp.einsum("bhsw,bhswd->bhsd", attn, vg)
        return (lambda x, *d: x.transpose(*d))(o, 0, 2, 1, 3).reshape(B, S, D) @ wo

    x = A_x
    g = _sigmoid((x * gate_w).sum(-1, keepdims=True))
    a = _A_ref(x, A_c_kv, A_w_q, A_w_uk, A_w_uv, A_w_o)
    b = _B_ref(x, B_wqkv, B_wo)
    return g * a + (1 - g) * b
```

```python
import functools
import numpy as np
import jax
import jax.numpy as jnp
from jax import lax
import jax.experimental.pallas as pl
import jax.experimental.pallas.tpu as pltpu

S = 2048
M = 1024
H = 32
D = 128
DC = 512
DH = 32
W = 8
DIL = 2
PAD = 16
BQ = 256
NQ = S // BQ
RB = 256
RI = 32
RO = 512
LOG2E = 1.4426950408889634
NT = (((1,), (1,)), ((), ()))
f32, bf16, u32 = jnp.float32, jnp.bfloat16, jnp.uint32


def _unpack(u):
    lo = lax.bitcast_convert_type(u << 16, f32)
    hi = lax.bitcast_convert_type(u & jnp.uint32(0xFFFF0000), f32)
    return lo, hi


def _kernel(x_hbm, ckv_hbm, wq_hbm, wuk_hbm, wuv_hbm, wo_hbm, wqkv_hbm, wob_hbm, gw_hbm, out_hbm,
            x_v, ckv_v, wq_v, wuk_v, wuv_v, wo_v, wqkv_v, wob_v, gw_v,
            wt_v, wtp_v, wobp_v, kb_v, vb_v, ob_v,
            q_v, k_v, v_v, s_v, ctx_v, out_v, sem, osem):
    copies = [
        pltpu.make_async_copy(wqkv_hbm, wqkv_v, sem.at[0]),
        pltpu.make_async_copy(x_hbm, x_v, sem.at[1]),
        pltpu.make_async_copy(gw_hbm, gw_v, sem.at[3]),
        pltpu.make_async_copy(ckv_hbm, ckv_v, sem.at[4]),
        pltpu.make_async_copy(wq_hbm.bitcast(u32), wq_v, sem.at[5]),
        pltpu.make_async_copy(wuk_hbm.bitcast(u32), wuk_v, sem.at[6]),
        pltpu.make_async_copy(wuv_hbm.bitcast(u32), wuv_v, sem.at[7]),
        pltpu.make_async_copy(wo_hbm, wo_v, sem.at[8]),
    ]
    wob_copies = [pltpu.make_async_copy(wob_hbm.bitcast(u32).at[:, t * 128:(t + 1) * 128], wob_v.at[t], sem.at[2])
                  for t in range(M // 128)]
    copies.insert(2, None)
    copies[0].start()
    copies[1].start()
    for c in wob_copies:
        c.start()
    for c in copies[3:]:
        c.start()

    copies[0].wait()
    for p in range(3):
        def tr_body(t, c):
            col = pl.multiple_of(p * M + t * 128, 128)
            blk = wqkv_v[:, pl.ds(col, 128)].astype(f32)
            blk_t = blk.T
            for mt in range(M // 128):
                wt_v[mt, pl.ds(pl.multiple_of(t * 128, 128), 128), :] = blk_t[:, mt * 128:(mt + 1) * 128]
            return c
        lax.fori_loop(0, M // 128, tr_body, 0)

        def perm_body(dh, c):
            for mt in range(M // 128):
                rows = wt_v[mt, pl.ds(dh, H, stride=DH), :]
                wtp_v[pl.ds(pl.multiple_of(p * M + dh * H, H), H), mt * 128:(mt + 1) * 128] = rows.astype(bf16)
            return c
        lax.fori_loop(0, DH, perm_body, 0)

    for c in wob_copies:
        c.wait()
    wob_u = wob_v

    def wob_body(j, c):
        r = pl.multiple_of(2 * j * H, 2 * H)
        for t in range(M // 128):
            lo, hi = _unpack(wob_u[t, pl.ds(j, H, stride=DH // 2), :])
            wobp_v[pl.ds(r, 2 * H), t * 128:(t + 1) * 128] = jnp.concatenate([lo, hi], axis=0).astype(bf16)
        return c
    lax.fori_loop(0, DH // 2, wob_body, 0)

    kb_v[0:PAD, :] = jnp.zeros((PAD, M), f32)
    vb_v[0:PAD, :] = jnp.zeros((PAD, M), f32)
    copies[1].wait()

    def b_proj(r0, n, p):
        return lax.dot_general(x_v[pl.ds(r0, n), :], wtp_v[p * M:(p + 1) * M, :], NT,
                               preferred_element_type=f32)

    def kv_body(i, c):
        r0 = pl.multiple_of(i * RO, RO)
        kb_v[pl.ds(PAD + r0, RO), :] = b_proj(r0, RO, 1)
        vb_v[pl.ds(PAD + r0, RO), :] = b_proj(r0, RO, 2)
        return c
    lax.fori_loop(0, S // RO, kv_body, 0)

    def b_chunk(i, first):
        r0 = i * RB if first else pl.multiple_of(i * RB, RB)
        q = b_proj(r0, RB, 0) * (DH ** -0.5 * LOG2E)
        kw = kb_v.at[pl.ds(r0, RB + PAD), :]
        vw = vb_v.at[pl.ds(r0, RB + PAD), :]
        for ib in range(RB // RI):
            qb = q[ib * RI:(ib + 1) * RI, :]
            base = ib * RI + PAD
            logits = []
            for w in range(W):
                pr = qb * kw[base - w * DIL:base - w * DIL + RI, :]
                acc = pr[:, 0:128]
                for t in range(1, M // 128):
                    acc = acc + pr[:, t * 128:(t + 1) * 128]
                acc = acc + pltpu.roll(acc, 64, 1)
                acc = acc + pltpu.roll(acc, 32, 1)
                if first and ib == 0 and w > 0:
                    pos = lax.broadcasted_iota(jnp.int32, (RI, 128), 0)
                    acc = jnp.where(pos >= w * DIL, acc, -1e9 * LOG2E)
                logits.append(acc)
            m = functools.reduce(jnp.maximum, logits)
            ps = [jnp.exp2(l - m) for l in logits]
            inv = 1.0 / functools.reduce(lambda a, b: a + b, ps)
            o = None
            for w in range(W):
                pw = ps[w] * inv
                term = jnp.concatenate([pw] * (M // 128), axis=1) * vw[base - w * DIL:base - w * DIL + RI, :]
                o = term if o is None else o + term
            ob_v[pl.ds(pl.multiple_of(r0 + ib * RI, RI), RI), :] = o.astype(bf16)

    b_chunk(0, True)

    def b_body(i, c):
        b_chunk(i, False)
        return c
    lax.fori_loop(1, S // RB, b_body, 0)

    for i in (4, 5, 6, 7):
        copies[i].wait()
    wq_u = wq_v
    wuk_u = wuk_v
    wuv_u = wuv_v

    def pair_w(ref_u, j, n):
        lo, hi = _unpack(ref_u[pl.ds(j, n, stride=H // 2), :])
        return lo.astype(bf16), hi.astype(bf16)

    def head_attn(e, h):
        for qi in range(NQ):
            sb = s_v.at[qi % 2]
            q = q_v[e, qi * BQ:(qi + 1) * BQ, :]
            m = None
            for c in range(qi + 1):
                s = lax.dot_general(q, k_v[e, c * BQ:(c + 1) * BQ, :], NT, preferred_element_type=f32)
                if c == qi:
                    row = lax.broadcasted_iota(jnp.int32, (BQ, BQ), 0)
                    col = lax.broadcasted_iota(jnp.int32, (BQ, BQ), 1)
                    s = jnp.where(col <= row, s, -1e9 * D ** -0.5 * LOG2E)
                sb[:, c * BQ:(c + 1) * BQ] = s
                for t in range(BQ // 128):
                    st = s[:, t * 128:(t + 1) * 128]
                    m = st if m is None else jnp.maximum(m, st)
            m = jnp.max(m, axis=1, keepdims=True)
            l = None
            acc = None
            for c in range(qi + 1):
                p = jnp.exp2(sb[:, c * BQ:(c + 1) * BQ] - m)
                for t in range(BQ // 128):
                    pt = p[:, t * 128:(t + 1) * 128]
                    l = pt if l is None else l + pt
                o = jnp.dot(p.astype(bf16), v_v[e, c * BQ:(c + 1) * BQ, :], preferred_element_type=f32)
                acc = o if acc is None else acc + o
            l = jnp.sum(l, axis=1, keepdims=True)
            ctx_v[h, qi * BQ:(qi + 1) * BQ, :] = (acc / l).astype(bf16)

    def pair_body(j, c):
        wq0, wq1 = pair_w(wq_u, j, M)
        q = jnp.dot(x_v[...], jnp.concatenate([wq0, wq1], axis=1), preferred_element_type=f32)
        q = (q * (D ** -0.5 * LOG2E)).astype(bf16)
        q_v[0] = q[:, :D]
        q_v[1] = q[:, D:]
        wk0, wk1 = pair_w(wuk_u, j, DC)
        wv0, wv1 = pair_w(wuv_u, j, DC)
        kv = jnp.dot(ckv_v[...], jnp.concatenate([wk0, wk1, wv0, wv1], axis=1),
                     preferred_element_type=f32).astype(bf16)
        k_v[0] = kv[:, 0 * D:1 * D]
        k_v[1] = kv[:, 1 * D:2 * D]
        v_v[0] = kv[:, 2 * D:3 * D]
        v_v[1] = kv[:, 3 * D:4 * D]

        def e_body(e, c2):
            head_attn(e, 2 * j + e)
            return c2
        lax.fori_loop(0, 2, e_body, 0)
        return c
    lax.fori_loop(0, H // 2, pair_body, 0)

    copies[3].wait()
    copies[8].wait()
    gw = gw_v[...].astype(f32)
    NO = S // RO

    def out_copy(i):
        return pltpu.make_async_copy(out_v.at[i % 2], out_hbm.at[pl.ds(i * RO, RO), :], osem.at[i % 2])

    for i in range(NO):
        rows = slice(i * RO, (i + 1) * RO)
        a = None
        for h in range(H):
            t = jnp.dot(ctx_v[h, rows, :], wo_v[h * D:(h + 1) * D, :], preferred_element_type=f32)
            a = t if a is None else a + t
        b = jnp.dot(ob_v[rows, :], wobp_v[...], preferred_element_type=f32)
        g = jax.nn.sigmoid(jnp.sum(x_v[rows, :].astype(f32) * gw, axis=1, keepdims=True))
        if i >= 2:
            out_copy(i - 2).wait()
        out_v[i % 2] = (g * a + (1.0 - g) * b).astype(bf16)
        out_copy(i).start()
    out_copy(NO - 2).wait()
    out_copy(NO - 1).wait()


@jax.jit
def pallas_gated_mix__compressed_kv_cla__sliding_local_dilated__prompt_kernel(
    A_x, A_c_kv, A_w_q, A_w_uk, A_w_uv, A_w_o, B_x, B_wqkv, B_wo, gate_w,
):
    del B_x
    any_spec = pl.BlockSpec(memory_space=pl.ANY)
    out = pl.pallas_call(
        _kernel,
        out_shape=jax.ShapeDtypeStruct((S, M), bf16),
        in_specs=[any_spec] * 9,
        out_specs=any_spec,
        scratch_shapes=[
            pltpu.VMEM((S, M), bf16), pltpu.VMEM((S, DC), bf16),
            pltpu.VMEM((M * H // 2, D), u32), pltpu.VMEM((DC * H // 2, D), u32), pltpu.VMEM((DC * H // 2, D), u32),
            pltpu.VMEM((H * D, M), bf16), pltpu.VMEM((M, 3 * M), bf16), pltpu.VMEM((M // 128, M // 2, 128), u32),
            pltpu.VMEM((1, M), bf16),
            pltpu.VMEM((M // 128, M, 128), f32), pltpu.VMEM((3 * M, M), bf16), pltpu.VMEM((M, M), bf16),
            pltpu.VMEM((S + PAD, M), f32), pltpu.VMEM((S + PAD, M), f32), pltpu.VMEM((S, M), bf16),
            pltpu.VMEM((2, S, D), bf16), pltpu.VMEM((2, S, D), bf16), pltpu.VMEM((2, S, D), bf16),
            pltpu.VMEM((2, BQ, S), f32), pltpu.VMEM((H, S, D), bf16), pltpu.VMEM((2, RO, M), bf16),
            pltpu.SemaphoreType.DMA((9,)), pltpu.SemaphoreType.DMA((2,)),
        ],
        compiler_params=pltpu.CompilerParams(vmem_limit_bytes=120 * 1024 * 1024),
    )(
        A_x.reshape(S, M), A_c_kv.reshape(S, DC), A_w_q.reshape(M * H, D), A_w_uk.reshape(DC * H, D),
        A_w_uv.reshape(DC * H, D), A_w_o.reshape(H * D, M), B_wqkv, B_wo, gate_w.reshape(1, M),
    )
    return out.reshape(1, S, M)
```

```python
import functools

import jax
import jax.numpy as jnp
from jax import lax
import jax.experimental.pallas as pl
import jax.experimental.pallas.tpu as pltpu

S = 2048
M = 1024
H = 32
D = 128
DC = 512
DH = 32
W = 8
DIL = 2
PAD = 16
PITCH = DH + 1
BQ = 256
NQ = S // BQ
NP = H // 2
RB = 512
NB = 512
RP = 512
RI = 16
RL = S // NP
RO = 512
LT = M // 128
LOG2E = 1.4426950408889634
NEG = -1e9
NT = (((1,), (1,)), ((), ()))
f32, bf16, u32 = jnp.float32, jnp.bfloat16, jnp.uint32


def _run(*lists):
    items = []
    for k, l in enumerate(lists):
        items += [((i + 0.5) / len(l), k, f) for i, f in enumerate(l)]
    items.sort(key=lambda t: (t[0], t[1]))
    for _, _, f in items:
        f()


def _unpack(u):
    lo = lax.bitcast_convert_type(u << 16, f32)
    hi = lax.bitcast_convert_type(u & jnp.uint32(0xFFFF0000), f32)
    return lo, hi


def _lane_tiles(x):
    return [x[:, t * 128:(t + 1) * 128] for t in range(x.shape[1] // 128)]


def _kernel(x_hbm, ckv_hbm, wq_hbm, wuk_hbm, wuv_hbm, wo_hbm, wqkv_hbm, wob_hbm, gw_hbm, out_hbm,
            x_v, ckv_v, wq_v, wuk_v, wuv_v, wo_v, gw_v, wobp_v, ob_v, qb_v, kb_v, vb_v,
            wa_v, wb_v, q_v, k_v, v_v, sem, osem):
    def cp(src, dst, i):
        return pltpu.make_async_copy(src, dst, sem.at[i])

    NX = S // RB
    x_cp = [cp(x_hbm.at[i * RB:(i + 1) * RB, :], x_v.at[i * RB:(i + 1) * RB, :], i) for i in range(NX)]
    gw_cp = cp(gw_hbm, gw_v, NX + 4)
    ckv_cp = cp(ckv_hbm, ckv_v, NX + 5)
    wq_cp = cp(wq_hbm.bitcast(u32), wq_v, NX + 6)
    wuk_cp = cp(wuk_hbm.bitcast(u32), wuk_v, NX + 7)
    wuv_cp = cp(wuv_hbm.bitcast(u32), wuv_v, NX + 8)
    wo_cp = cp(wo_hbm, wo_v, NX + 9)

    def wprep_steps(j):
        def one(src, dst, r0, n, c0, c1):
            def f():
                lo, hi = _unpack(src[pl.ds(r0 * NP + j, n, stride=NP), :])
                dst[r0:r0 + n, c0:c0 + D] = lo.astype(bf16)
                dst[r0:r0 + n, c1:c1 + D] = hi.astype(bf16)
            return f
        n = 256
        return ([one(wq_v, wa_v, r0, n, 0, D) for r0 in range(0, M, n)]
                + [one(wuk_v, wb_v, r0, n, 0, D) for r0 in range(0, DC, n)]
                + [one(wuv_v, wb_v, r0, n, 2 * D, 3 * D) for r0 in range(0, DC, n)])

    def aproj_steps(base, rows):
        def kv_piece(r0):
            def f():
                r = pl.ds(base + r0, RP)
                y = jnp.dot(ckv_v[r, :], wb_v[...], preferred_element_type=f32).astype(bf16)
                k_v[0, r, :] = y[:, 0 * D:1 * D]
                k_v[1, r, :] = y[:, 1 * D:2 * D]
                v_v[0, r, :] = y[:, 2 * D:3 * D]
                v_v[1, r, :] = y[:, 3 * D:4 * D]
            return f

        def q_piece(r0):
            def f():
                r = pl.ds(base + r0, RP)
                y = jnp.dot(x_v[r, :], wa_v[...], preferred_element_type=f32)
                y = (y * (D ** -0.5 * LOG2E)).astype(bf16)
                q_v[0, r, :] = y[:, :D]
                q_v[1, r, :] = y[:, D:]
            return f
        return [kv_piece(r0) for r0 in range(0, rows, RP)] + [q_piece(r0) for r0 in range(0, rows, RP)]

    def local_steps(r0, rows):
        def block(ib):
            def f():
                r = r0 + ib * RI
                qt = [qb_v[t, pl.ds(r, RI), :] for t in range(LT)]
                pos = r + lax.broadcasted_iota(jnp.int32, (RI, 128), 0)
                logits = []
                for w in range(W):
                    acc = None
                    for t in range(LT):
                        pr = qt[t] * kb_v[t, pl.ds(r + PAD - w * DIL, RI), :]
                        acc = pr if acc is None else acc + pr
                    acc = acc + pltpu.roll(acc, 64, 1)
                    acc = acc + pltpu.roll(acc, 32, 1)
                    if w > 0:
                        acc = jnp.where(pos >= w * DIL, acc, NEG * LOG2E)
                    logits.append(acc)
                m = functools.reduce(jnp.maximum, logits)
                ps = [jnp.exp2(l - m) for l in logits]
                inv = 1.0 / functools.reduce(lambda a, b: a + b, ps)
                ps = [p * inv for p in ps]
                for t in range(LT):
                    o = None
                    for w in range(W):
                        term = ps[w] * vb_v[t, pl.ds(r + PAD - w * DIL, RI), :]
                        o = term if o is None else o + term
                    ob_v[pl.ds(pl.multiple_of(r, RI), RI), t * 128:(t + 1) * 128] = o.astype(bf16)
            return f
        return [block(ib) for ib in range(rows // RI)]

    def phase1(wqkv_v, wob_v, wt_v, wtp_v):
        wqkv_cp = [cp(wqkv_hbm.at[:, p * M:(p + 1) * M], wqkv_v.at[:, p * M:(p + 1) * M], NX + p)
                   for p in range(3)]
        wob_cp = [cp(wob_hbm.bitcast(u32).at[:, t * 128:(t + 1) * 128], wob_v.at[t], NX + 3) for t in range(LT)]
        for c in [wqkv_cp[1], x_cp[0], wqkv_cp[2]] + x_cp[1:] + [wqkv_cp[0]] + wob_cp + [
                wq_cp, wuk_cp, wuv_cp, ckv_cp, wo_cp, gw_cp]:
            c.start()

        def prep_steps(p):
            def tr(t):
                def f():
                    if t == 0:
                        wqkv_cp[p].wait()
                    blk_t = wqkv_v[:, p * M + t * 128:p * M + (t + 1) * 128].astype(f32).T
                    for hl in range(128 // DH):
                        r = (t * (128 // DH) + hl) * PITCH
                        for mt in range(LT):
                            wt_v[mt, r:r + DH, :] = blk_t[hl * DH:(hl + 1) * DH, mt * 128:(mt + 1) * 128]
                return f

            def perm(d0):
                def f():
                    for dh in range(d0, d0 + 4):
                        for mt in range(LT):
                            rows = wt_v[mt, pl.ds(dh, H, stride=PITCH), :]
                            wtp_v[p * M + dh * H:p * M + (dh + 1) * H, mt * 128:(mt + 1) * 128] = rows.astype(bf16)
                return f
            return [tr(t) for t in range(LT)] + [perm(d0) for d0 in range(0, DH, 4)]

        def proj_steps(p):
            def piece(i, c0):
                def f():
                    if p == 1 and c0 == 0:
                        x_cp[i].wait()
                    r0 = i * RB
                    y = lax.dot_general(x_v[r0:r0 + RB, :], wtp_v[p * M + c0:p * M + c0 + NB, :], NT,
                                        preferred_element_type=f32)
                    if p == 0:
                        y = y * (DH ** -0.5 * LOG2E)
                    for t, yt in enumerate(_lane_tiles(y)):
                        if p == 0:
                            qb_v[c0 // 128 + t, r0:r0 + RB, :] = yt
                        elif p == 1:
                            kb_v[c0 // 128 + t, PAD + r0:PAD + r0 + RB, :] = yt
                        else:
                            vb_v[c0 // 128 + t, PAD + r0:PAD + r0 + RB, :] = yt
                return f
            return [piece(i, c0) for i in range(NX) for c0 in range(0, M, NB)]

        def wob_steps():
            def one(j):
                def f():
                    if j == 0:
                        for c in wob_cp:
                            c.wait()
                    for t in range(LT):
                        lo, hi = _unpack(wob_v[t, pl.ds(j, H, stride=DH // 2), :])
                        wobp_v[2 * j * H:(2 * j + 2) * H, t * 128:(t + 1) * 128] = (
                            jnp.concatenate([lo, hi], axis=0).astype(bf16))
                return f
            return [one(j) for j in range(DH // 2)]

        kb_v[:, 0:PAD, :] = jnp.zeros((LT, PAD, 128), f32)
        vb_v[:, 0:PAD, :] = jnp.zeros((LT, PAD, 128), f32)
        _run(prep_steps(1))
        _run(proj_steps(1), prep_steps(2))
        _run(proj_steps(2), prep_steps(0))

        def waits():
            for c in (wq_cp, wuk_cp, wuv_cp, ckv_cp):
                c.wait()
        _run(proj_steps(0), wob_steps() + [waits] + wprep_steps(0))

    pl.run_scoped(phase1, pltpu.VMEM((M, 3 * M), bf16), pltpu.VMEM((LT, M // 2, 128), u32),
                  pltpu.VMEM((LT, H * PITCH, 128), f32), pltpu.VMEM((3 * M, M), bf16))

    def phase23(s_v, ctx_v, out_v):
        HB = BQ // 2

        def attn_steps(j):
            orders = '76543210,76543210'.split(',')
            tasks = [(e, int(ch)) for e in range(2) for ch in orders[e]]
            rowmax = {}

            def p1_steps(n):
                e, qi = tasks[n]
                sb = s_v.at[n % 2]
                r0 = qi * BQ
                state = {"m": None}

                def upd(m, s):
                    for x in _lane_tiles(s):
                        m = x if m is None else jnp.maximum(m, x)
                    return m

                def full(c):
                    def f():
                        s = lax.dot_general(q_v[e, r0:r0 + BQ, :], k_v[e, c * BQ:(c + 1) * BQ, :], NT,
                                            preferred_element_type=f32)
                        sb[:, c * BQ:(c + 1) * BQ] = s
                        state["m"] = upd(state["m"], s)
                    return f

                def diag():
                    neg = NEG * D ** -0.5 * LOG2E
                    tri = (lax.broadcasted_iota(jnp.int32, (HB, HB), 1)
                           <= lax.broadcasted_iota(jnp.int32, (HB, HB), 0))
                    s0 = lax.dot_general(q_v[e, r0:r0 + HB, :], k_v[e, r0:r0 + HB, :], NT,
                                         preferred_element_type=f32)
                    s0 = jnp.where(tri, s0, neg)
                    s1 = lax.dot_general(q_v[e, r0 + HB:r0 + BQ, :], k_v[e, r0:r0 + BQ, :], NT,
                                         preferred_element_type=f32)
                    s1 = jnp.concatenate([s1[:, :HB], jnp.where(tri, s1[:, HB:], neg)], axis=1)
                    sb[0:HB, r0:r0 + HB] = s0
                    sb[HB:BQ, r0:r0 + BQ] = s1
                    md = jnp.concatenate([upd(None, s0), upd(None, s1)], axis=0)
                    m = md if state["m"] is None else jnp.maximum(state["m"], md)
                    rowmax[n] = jnp.max(m, axis=1, keepdims=True)
                return [full(c) for c in range(qi)] + [diag]

            def p2_steps(n):
                e, qi = tasks[n]
                sb = s_v.at[n % 2]
                r0 = qi * BQ
                state = {"l": None, "acc": None}

                def lsum(l, p):
                    for x in _lane_tiles(p):
                        l = x if l is None else l + x
                    return l

                def full(c):
                    def f():
                        p = jnp.exp2(sb[:, c * BQ:(c + 1) * BQ] - rowmax[n])
                        state["l"] = lsum(state["l"], p)
                        o = jnp.dot(p.astype(bf16), v_v[e, c * BQ:(c + 1) * BQ, :],
                                    preferred_element_type=f32)
                        state["acc"] = o if state["acc"] is None else state["acc"] + o
                    return f

                def diag():
                    m = rowmax[n]
                    p0 = jnp.exp2(sb[0:HB, r0:r0 + HB] - m[:HB])
                    p1 = jnp.exp2(sb[HB:BQ, r0:r0 + BQ] - m[HB:])
                    o0 = jnp.dot(p0.astype(bf16), v_v[e, r0:r0 + HB, :], preferred_element_type=f32)
                    o1 = jnp.dot(p1.astype(bf16), v_v[e, r0:r0 + BQ, :], preferred_element_type=f32)
                    l = jnp.concatenate([lsum(None, p0), lsum(None, p1)], axis=0)
                    acc = jnp.concatenate([o0, o1], axis=0)
                    if state["l"] is not None:
                        l = l + state["l"]
                        acc = acc + state["acc"]
                    l = jnp.sum(l, axis=1, keepdims=True)
                    if '1' == '1':
                        inv = pl.reciprocal(l, approx=True)
                        inv = inv * (2.0 - l * inv)
                        ctx_v[2 * j + e, r0:r0 + BQ, :] = (acc * inv).astype(bf16)
                    else:
                        ctx_v[2 * j + e, r0:r0 + BQ, :] = (acc / l).astype(bf16)
                return [full(c) for c in range(qi)] + [diag]

            steps = p1_steps(0)
            for n in range(len(tasks)):
                b = p2_steps(n)
                a = p1_steps(n + 1) if n + 1 < len(tasks) else []
                for i in range(max(len(a), len(b))):
                    steps += a[i:i + 1] + b[i:i + 1]
            return steps

        NI = 2

        def proj_body(j):
            def body(i, c):
                base = pl.multiple_of(i * (S // NI), S // NI)
                r0 = pl.multiple_of(j * RL + i * (RL // NI), RL // NI)
                _run(aproj_steps(base, S // NI), local_steps(r0, RL // NI))
                return c
            return body

        def pair_body(j, c):
            lax.fori_loop(0, NI, proj_body(j), 0)
            _run(attn_steps(j), wprep_steps(jnp.minimum(j + 1, NP - 1)))
            return c

        lax.fori_loop(0, NP, pair_body, 0)

        gw_cp.wait()
        wo_cp.wait()
        gw = gw_v[...].astype(f32)
        NO = S // RO

        def out_copy(i):
            return pltpu.make_async_copy(out_v.at[i % 2], out_hbm.at[pl.ds(i * RO, RO), :], osem.at[i % 2])

        for i in range(NO):
            rows = slice(i * RO, (i + 1) * RO)
            a = None
            for h in range(H):
                t = jnp.dot(ctx_v[h, rows, :], wo_v[h * D:(h + 1) * D, :], preferred_element_type=f32)
                a = t if a is None else a + t
            b = jnp.dot(ob_v[rows, :], wobp_v[...], preferred_element_type=f32)
            g = jax.nn.sigmoid(jnp.sum(x_v[rows, :].astype(f32) * gw, axis=1, keepdims=True))
            if i >= 2:
                out_copy(i - 2).wait()
            out_v[i % 2] = (g * a + (1.0 - g) * b).astype(bf16)
            out_copy(i).start()
        out_copy(NO - 2).wait()
        out_copy(NO - 1).wait()

    pl.run_scoped(phase23, pltpu.VMEM((2, BQ, S), f32), pltpu.VMEM((H, S, D), bf16), pltpu.VMEM((2, RO, M), bf16))


@jax.jit
def pallas_gated_mix__compressed_kv_cla__sliding_local_dilated__prompt_kernel(
    A_x, A_c_kv, A_w_q, A_w_uk, A_w_uv, A_w_o, B_x, B_wqkv, B_wo, gate_w,
):
    del B_x
    any_spec = pl.BlockSpec(memory_space=pl.ANY)
    out = pl.pallas_call(
        _kernel,
        out_shape=jax.ShapeDtypeStruct((S, M), bf16),
        in_specs=[any_spec] * 9,
        out_specs=any_spec,
        scratch_shapes=[
            pltpu.VMEM((S, M), bf16), pltpu.VMEM((S, DC), bf16),
            pltpu.VMEM((M * NP, D), u32), pltpu.VMEM((DC * NP, D), u32), pltpu.VMEM((DC * NP, D), u32),
            pltpu.VMEM((H * D, M), bf16), pltpu.VMEM((1, M), bf16), pltpu.VMEM((M, M), bf16),
            pltpu.VMEM((S, M), bf16),
            pltpu.VMEM((LT, S, 128), f32), pltpu.VMEM((LT, S + PAD, 128), f32), pltpu.VMEM((LT, S + PAD, 128), f32),
            pltpu.VMEM((M, 2 * D), bf16), pltpu.VMEM((DC, 4 * D), bf16),
            pltpu.VMEM((2, S, D), bf16), pltpu.VMEM((2, S, D), bf16), pltpu.VMEM((2, S, D), bf16),
            pltpu.SemaphoreType.DMA((S // RB + 10,)), pltpu.SemaphoreType.DMA((2,)),
        ],
        compiler_params=pltpu.CompilerParams(vmem_limit_bytes=120 * 1024 * 1024),
    )(
        A_x.reshape(S, M), A_c_kv.reshape(S, DC), A_w_q.reshape(M * H, D), A_w_uk.reshape(DC * H, D),
        A_w_uv.reshape(DC * H, D), A_w_o.reshape(H * D, M), B_wqkv, B_wo, gate_w.reshape(1, M),
    )
    return out.reshape(1, S, M)
```

```python
import functools

import jax
import jax.numpy as jnp
from jax import lax
import jax.experimental.pallas as pl
import jax.experimental.pallas.tpu as pltpu

S = 2048
M = 1024
H = 32
D = 128
DC = 512
DH = 32
W = 8
DIL = 2
PAD = 16
PITCH = DH + 1
BQ = 256
NQ = S // BQ
NP = H // 2
RB = 512
NB = 512
RP = 512
RI = 16
RL = S // NP
RO = 2048
CW = 256
DIAG = 1
NS = 2
LAG = 1
PINP = 3
PINL = 1
PINW = 0
WP = H // 2 + 1
CO = 512
ALL = slice(None)
LT = M // 128
LOG2E = 1.4426950408889634
NEG = -1e9
NT = (((1,), (1,)), ((), ()))
f32, bf16, u32 = jnp.float32, jnp.bfloat16, jnp.uint32


def _run(*lists):
    items = []
    for k, l in enumerate(lists):
        items += [((i + 0.5) / len(l), k, f) for i, f in enumerate(l)]
    items.sort(key=lambda t: (t[0], t[1]))
    for _, _, f in items:
        f()


def _unpack(u):
    lo = lax.bitcast_convert_type(u << 16, f32)
    hi = lax.bitcast_convert_type(u & jnp.uint32(0xFFFF0000), f32)
    return lo, hi


def _half(rows):
    if isinstance(rows, slice):
        return slice(rows.start // 2, rows.stop // 2)
    start = rows.start // 2
    return pl.ds(start if isinstance(start, int) else pl.multiple_of(start, 8), rows.size // 2)


def _ld(ref, rows, cols=slice(None)):
    return pltpu.bitcast(ref[_half(rows), cols], bf16)


def _st(ref, rows, cols, val):
    ref[_half(rows), cols] = pltpu.bitcast(val, u32)


def _lane_tiles(x):
    return [x[:, t * 128:(t + 1) * 128] for t in range(x.shape[1] // 128)]


def _kernel(x_hbm, ckv_hbm, wq_hbm, wuk_hbm, wuv_hbm, wo_hbm, wqkv_hbm, wob_hbm, gw_hbm, out_hbm,
            x_v, ckv_v, wq_v, wuk_v, wuv_v, wo_v, gw_v, wobp_v, ob_v, qb_v, kb_v, vb_v,
            wa_v, wb_v, q_v, k_v, v_v, zero_s, sem, osem):
    zero_s[0] = 0
    toks = []

    def pin(lhs):
        if not toks:
            return lhs
        tok = functools.reduce(lambda a, b: a | b, toks)
        toks.clear()
        never = (lax.broadcasted_iota(jnp.int32, (8, 128), 1) + zero_s[0]) < 0
        head = pltpu.bitcast(lhs[0:16, 0:128], u32)
        head = pltpu.bitcast(jnp.where(never, tok, head), bf16)
        top = head if lhs.shape[1] == 128 else jnp.concatenate([head, lhs[0:16, 128:]], axis=1)
        return jnp.concatenate([top, lhs[16:]], axis=0)

    def cp(src, dst, i):
        return pltpu.make_async_copy(src, dst, sem.at[i])

    NX = S // RB
    HR = RB // 2
    x_cp = [cp(x_hbm.bitcast(u32).at[i * HR:(i + 1) * HR, :], x_v.at[i * HR:(i + 1) * HR, :], i) for i in range(NX)]
    gw_cp = cp(gw_hbm, gw_v, NX + 4)
    ckv_cp = cp(ckv_hbm.bitcast(u32), ckv_v, NX + 5)
    def w_cps(src, dst, i):
        return [cp(src.bitcast(u32).at[:, c], dst.at[:, c * WP:c * WP + NP, :], i) for c in range(8)]
    wq_cp = w_cps(wq_hbm, wq_v, NX + 6)
    wuk_cp = w_cps(wuk_hbm, wuk_v, NX + 7)
    wuv_cp = w_cps(wuv_hbm, wuv_v, NX + 8)
    wo_cp = cp(wo_hbm.bitcast(u32), wo_v, NX + 9)

    def wprep_steps(j, tok=False):
        def one(src, dst, r0, n, c0, c1):
            def f():
                u = [src[g, pl.ds(j, 8, stride=WP), :] for g in range(r0 // 8, (r0 + n) // 8)]
                lo, hi = _unpack(jnp.concatenate(u, axis=0))
                lo, hi = lo.astype(bf16), hi.astype(bf16)
                _st(dst, slice(r0, r0 + n), slice(c0, c0 + D), lo)
                _st(dst, slice(r0, r0 + n), slice(c1, c1 + D), hi)
                if PINW and tok:
                    toks.extend(pltpu.bitcast(x[i:i + 16], u32) for x in (lo, hi) for i in range(0, n, 16))
            return f
        n = 256
        return ([one(wq_v, wa_v, r0, n, 0, D) for r0 in range(0, M, n)]
                + [one(wuk_v, wb_v, r0, n, 0, D) for r0 in range(0, DC, n)]
                + [one(wuv_v, wb_v, r0, n, 2 * D, 3 * D) for r0 in range(0, DC, n)])

    def aproj_steps(base, rows):
        def kv_piece(r0):
            def f():
                r = pl.ds(pl.multiple_of(base + r0, RP), RP)
                y = jnp.dot(pin(_ld(ckv_v, r)), _ld(wb_v, slice(0, DC)), preferred_element_type=f32).astype(bf16)
                _st(k_v.at[0], r, ALL, y[:, 0 * D:1 * D])
                _st(k_v.at[1], r, ALL, y[:, 1 * D:2 * D])
                _st(v_v.at[0], r, ALL, y[:, 2 * D:3 * D])
                _st(v_v.at[1], r, ALL, y[:, 3 * D:4 * D])
            return f

        def q_piece(r0):
            def f():
                r = pl.ds(pl.multiple_of(base + r0, RP), RP)
                y = jnp.dot(pin(_ld(x_v, r)), _ld(wa_v, slice(0, M)), preferred_element_type=f32)
                y = (y * (D ** -0.5 * LOG2E)).astype(bf16)
                _st(q_v.at[0], r, ALL, y[:, :D])
                _st(q_v.at[1], r, ALL, y[:, D:])
            return f
        return [kv_piece(r0) for r0 in range(0, rows, RP)] + [q_piece(r0) for r0 in range(0, rows, RP)]

    def local_steps(r0, rows):
        def block(ib):
            def f():
                r = r0 + ib * RI
                qt = [qb_v[t, pl.ds(r, RI), :] for t in range(LT)]
                pos = r + lax.broadcasted_iota(jnp.int32, (RI, 128), 0)
                logits = []
                for w in range(W):
                    acc = None
                    for t in range(LT):
                        pr = qt[t] * kb_v[t, pl.ds(r + PAD - w * DIL, RI), :]
                        acc = pr if acc is None else acc + pr
                    acc = acc + pltpu.roll(acc, 64, 1)
                    acc = acc + pltpu.roll(acc, 32, 1)
                    if w > 0:
                        acc = jnp.where(pos >= w * DIL, acc, NEG * LOG2E)
                    logits.append(acc)
                m = functools.reduce(jnp.maximum, logits)
                ps = [jnp.exp2(l - m) for l in logits]
                inv = 1.0 / functools.reduce(lambda a, b: a + b, ps)
                ps = [p * inv for p in ps]
                for t in range(LT):
                    o = None
                    for w in range(W):
                        term = ps[w] * vb_v[t, pl.ds(r + PAD - w * DIL, RI), :]
                        o = term if o is None else o + term
                    ob = o.astype(bf16)
                    _st(ob_v, pl.ds(r, RI), slice(t * 128, (t + 1) * 128), ob)
                    if PINL:
                        toks.append(pltpu.bitcast(ob[0:16], u32))
            return f
        return [block(ib) for ib in range(rows // RI)]

    def phase1(wqkv_v, wob_v, wt_v, wtp_v):
        def wcols(c0, n, i):
            return cp(wqkv_hbm.at[:, c0:c0 + n], wqkv_v.at[:, c0:c0 + n], i)
        wk_cp = [wcols(M + t * 128, 128, NX + 10 + t) for t in range(LT)]
        wqkv_cp = [wcols(0, M, NX), None, wcols(2 * M, M, NX + 2)]
        wob_cp = [cp(wob_hbm.bitcast(u32).at[:, t * 128:(t + 1) * 128], wob_v.at[t], NX + 3) for t in range(LT)]
        third = wob_cp + wq_cp + wuk_cp + wuv_cp + [ckv_cp, wo_cp, gw_cp]
        OR = '1'
        if OR == '0':
            lst = wk_cp + [x_cp[0], wqkv_cp[2]] + x_cp[1:] + [wqkv_cp[0]]
        elif OR == '1':
            lst = wk_cp + [x_cp[0], x_cp[1], wqkv_cp[2]] + x_cp[2:] + [wqkv_cp[0]]
        else:
            lst = [x_cp[0]] + wk_cp + [x_cp[1], wqkv_cp[2]] + x_cp[2:] + [wqkv_cp[0]]
        for c in lst:
            c.start()
        T3 = 3

        def prep_steps(p):
            def tr(t):
                def f():
                    if p == 1:
                        wk_cp[t].wait()
                    elif t == 0:
                        wqkv_cp[p].wait()
                    blk_t = wqkv_v[:, p * M + t * 128:p * M + (t + 1) * 128].astype(f32).T
                    for hl in range(128 // DH):
                        r = (t * (128 // DH) + hl) * PITCH
                        for mt in range(LT):
                            wt_v[mt, r:r + DH, :] = blk_t[hl * DH:(hl + 1) * DH, mt * 128:(mt + 1) * 128]
                return f

            def perm(d0):
                def f():
                    for dh in range(d0, d0 + 4):
                        for mt in range(LT):
                            rows = wt_v[mt, pl.ds(dh, H, stride=PITCH), :]
                            rows = rows.astype(bf16)
                            _st(wtp_v, slice(p * M + dh * H, p * M + (dh + 1) * H), slice(mt * 128, (mt + 1) * 128), rows)
                            if PINP and p != 1:
                                toks.extend(pltpu.bitcast(rows[i:i + 16], u32) for i in range(0, H, 16))
                return f
            return [tr(t) for t in range(LT)] + [perm(d0) for d0 in range(0, DH, 4)]

        def proj_steps(p):
            def piece(i, c0):
                def f():
                    if p == 1 and c0 == 0:
                        x_cp[i].wait()
                        if i == T3:
                            for c in third:
                                c.start()
                    r0 = i * RB
                    y = lax.dot_general(pin(_ld(x_v, slice(r0, r0 + RB))), _ld(wtp_v, slice(p * M + c0, p * M + c0 + NB)), NT,
                                        preferred_element_type=f32)
                    if p == 0:
                        y = y * (DH ** -0.5 * LOG2E)
                    for t, yt in enumerate(_lane_tiles(y)):
                        if p == 0:
                            qb_v[c0 // 128 + t, r0:r0 + RB, :] = yt
                        elif p == 1:
                            kb_v[c0 // 128 + t, PAD + r0:PAD + r0 + RB, :] = yt
                        else:
                            vb_v[c0 // 128 + t, PAD + r0:PAD + r0 + RB, :] = yt
                return f
            return [piece(i, c0) for i in range(NX) for c0 in range(0, M, NB)]

        def wob_steps():
            def one(j):
                def f():
                    if j == 0:
                        for c in wob_cp:
                            c.wait()
                    for t in range(LT):
                        lo, hi = _unpack(wob_v[t, pl.ds(j, H, stride=DH // 2), :])
                        rows = jnp.concatenate([lo, hi], axis=0).astype(bf16)
                        _st(wobp_v, slice(2 * j * H, (2 * j + 2) * H), slice(t * 128, (t + 1) * 128), rows)
                        if PINP & 2:
                            toks.extend(pltpu.bitcast(rows[i:i + 16], u32) for i in range(0, 2 * H, 16))
                return f
            return [one(j) for j in range(DH // 2)]

        kb_v[:, 0:PAD, :] = jnp.zeros((LT, PAD, 128), f32)
        vb_v[:, 0:PAD, :] = jnp.zeros((LT, PAD, 128), f32)
        pk = prep_steps(1)
        _run(pk[:LT])
        _run(pk[LT:])
        pj = proj_steps(1)
        pv = prep_steps(2)
        KS = 2
        per = len(pj) // NX
        for i in range(NX):
            if i < KS:
                _run(pj[i * per:(i + 1) * per])
            else:
                n0, n1 = [len(pv) * (ii - KS) // (NX - KS) for ii in (i, i + 1)]
                _run(pj[i * per:(i + 1) * per], pv[n0:n1])
        _run(proj_steps(2), prep_steps(0))

        def waits():
            for c in wq_cp + wuk_cp + wuv_cp + [ckv_cp]:
                c.wait()
        _run(proj_steps(0), wob_steps() + [waits] + wprep_steps(0))
        toks.clear()

    pl.run_scoped(phase1, pltpu.VMEM((M, 3 * M), bf16), pltpu.VMEM((LT, M // 2, 128), u32),
                  pltpu.VMEM((LT, H * PITCH, 128), f32), pltpu.VMEM((3 * M // 2, M), u32))

    def phase23(s_v, ctx_v, out_v):
        HB = BQ // 2

        def attn_steps(j):
            orders = '76543210,76543210'.split(',')
            tasks = [(e, int(ch)) for e in range(2) for ch in orders[e]]
            rowmax = {}

            def segments(qi):
                segs, k0 = [], 0
                while k0 < qi * BQ:
                    wd = CW if k0 + CW <= qi * BQ else BQ
                    segs.append((k0, wd))
                    k0 += wd
                return segs

            def p1_steps(n):
                e, qi = tasks[n]
                sb = s_v.at[n % NS]
                r0 = qi * BQ
                state = {"m": None}

                def upd(m, s):
                    for x in _lane_tiles(s):
                        m = x if m is None else jnp.maximum(m, x)
                    return m

                def full(k0, wd):
                    def f():
                        s = lax.dot_general(pin(_ld(q_v.at[e], slice(r0, r0 + BQ))), _ld(k_v.at[e], slice(k0, k0 + wd)), NT,
                                            preferred_element_type=f32)
                        sb[:, k0:k0 + wd] = s
                        state["m"] = upd(state["m"], s)
                    return f

                def diag():
                    neg = NEG * D ** -0.5 * LOG2E
                    if DIAG == 0:
                        tri = (lax.broadcasted_iota(jnp.int32, (BQ, BQ), 1)
                               <= lax.broadcasted_iota(jnp.int32, (BQ, BQ), 0))
                        s = lax.dot_general(_ld(q_v.at[e], slice(r0, r0 + BQ)), _ld(k_v.at[e], slice(r0, r0 + BQ)), NT,
                                            preferred_element_type=f32)
                        s = jnp.where(tri, s, neg)
                        sb[:, r0:r0 + BQ] = s
                        md = upd(None, s)
                    else:
                        tri = (lax.broadcasted_iota(jnp.int32, (HB, HB), 1)
                               <= lax.broadcasted_iota(jnp.int32, (HB, HB), 0))
                        sa = lax.dot_general(_ld(q_v.at[e], slice(r0, r0 + BQ)), _ld(k_v.at[e], slice(r0, r0 + HB)), NT,
                                             preferred_element_type=f32)
                        sa = jnp.concatenate([jnp.where(tri, sa[:HB], neg), sa[HB:]], axis=0)
                        sc = lax.dot_general(_ld(q_v.at[e], slice(r0 + HB, r0 + BQ)), _ld(k_v.at[e], slice(r0 + HB, r0 + BQ)), NT,
                                             preferred_element_type=f32)
                        sc = jnp.where(tri, sc, neg)
                        sb[:, r0:r0 + HB] = sa
                        sb[HB:BQ, r0 + HB:r0 + BQ] = sc
                        md = jnp.concatenate([sa[:HB], jnp.maximum(sa[HB:], sc)], axis=0)
                    m = md if state["m"] is None else jnp.maximum(state["m"], md)
                    rowmax[n] = jnp.max(m, axis=1, keepdims=True)
                return [full(*sg) for sg in segments(qi)] + [diag]

            def p2_steps(n):
                e, qi = tasks[n]
                sb = s_v.at[n % NS]
                r0 = qi * BQ
                state = {"l": None, "acc": None}

                def lsum(l, p):
                    t = None
                    for x in _lane_tiles(p):
                        t = x if t is None else t + x
                    return t if l is None else l + t

                def full(k0, wd):
                    def f():
                        p = jnp.exp2(sb[:, k0:k0 + wd] - rowmax[n])
                        state["l"] = lsum(state["l"], p)
                        o = jnp.dot(p.astype(bf16), _ld(v_v.at[e], slice(k0, k0 + wd)), preferred_element_type=f32)
                        state["acc"] = o if state["acc"] is None else state["acc"] + o
                    return f

                def diag():
                    m = rowmax[n]
                    if DIAG == 0:
                        p = jnp.exp2(sb[:, r0:r0 + BQ] - m)
                        l = lsum(None, p)
                        acc = jnp.dot(p.astype(bf16), _ld(v_v.at[e], slice(r0, r0 + BQ)), preferred_element_type=f32)
                    else:
                        pa = jnp.exp2(sb[:, r0:r0 + HB] - m)
                        pc = jnp.exp2(sb[HB:BQ, r0 + HB:r0 + BQ] - m[HB:])
                        oa = jnp.dot(pa.astype(bf16), _ld(v_v.at[e], slice(r0, r0 + HB)), preferred_element_type=f32)
                        oc = jnp.dot(pc.astype(bf16), _ld(v_v.at[e], slice(r0 + HB, r0 + BQ)), preferred_element_type=f32)
                        l = jnp.concatenate([pa[:HB], pa[HB:] + pc], axis=0)
                        acc = jnp.concatenate([oa[:HB], oa[HB:] + oc], axis=0)
                    if state["l"] is not None:
                        l = l + state["l"]
                        acc = acc + state["acc"]
                    l = jnp.sum(l, axis=1, keepdims=True)
                    inv = pl.reciprocal(l, approx=True)
                    inv = inv * (2.0 - l * inv)
                    _st(ctx_v.at[2 * j + e], slice(r0, r0 + BQ), ALL, (acc * inv).astype(bf16))
                return [full(*sg) for sg in segments(qi)] + [diag]

            sa = [(n, f) for n in range(len(tasks)) for f in p1_steps(n)]
            sb_ = [(n, f) for n in range(len(tasks)) for f in p2_steps(n)]
            end_a = {n: i + 1 for i, (n, _) in enumerate(sa)}
            end_b = {n: i + 1 for i, (n, _) in enumerate(sb_)}
            steps, ia, ib, last = [], 0, 0, "b"
            while ia < len(sa) or ib < len(sb_):
                can_a = ia < len(sa) and (sa[ia][0] < NS or ib >= end_b[sa[ia][0] - NS])
                can_b = ib < len(sb_) and (ia >= min(end_a[sb_[ib][0]] + LAG, len(sa)) or not can_a)
                if can_a and (last == "b" or not can_b):
                    steps.append(sa[ia][1])
                    ia, last = ia + 1, "a"
                else:
                    assert ia >= end_a[sb_[ib][0]]
                    steps.append(sb_[ib][1])
                    ib, last = ib + 1, "b"
            return steps

        NI = 2

        def proj_body(j):
            def body(i, c):
                base = pl.multiple_of(i * (S // NI), S // NI)
                r0 = pl.multiple_of(j * RL + i * (RL // NI), RL // NI)
                _run(aproj_steps(base, S // NI), local_steps(r0, RL // NI))
                toks.clear()
                return c
            return body

        def pair_body(j, c):
            lax.fori_loop(0, NI, proj_body(j), 0)
            _run(attn_steps(j), wprep_steps(jnp.minimum(j + 1, NP - 1), True))
            toks.clear()
            return c

        lax.fori_loop(0, NP, pair_body, 0)

        gw_cp.wait()
        wo_cp.wait()
        gw = gw_v[...].astype(f32)
        blocks = [(r, c) for r in range(0, S, RO) for c in range(0, M, CO)]

        def out_copy(i):
            r, c = blocks[i]
            return pltpu.make_async_copy(out_v.at[i % 2], out_hbm.at[r:r + RO, c:c + CO], osem.at[i % 2])

        g = None
        for i, (r, c) in enumerate(blocks):
            rows, cols = slice(r, r + RO), slice(c, c + CO)
            if c == 0:
                g = jax.nn.sigmoid(jnp.sum(_ld(x_v, rows).astype(f32) * gw, axis=1, keepdims=True))
            a = None
            for h in range(H):
                t = jnp.dot(_ld(ctx_v.at[h], rows), _ld(wo_v, slice(h * D, (h + 1) * D), cols),
                            preferred_element_type=f32)
                a = t if a is None else a + t
            b = jnp.dot(_ld(ob_v, rows), _ld(wobp_v, slice(0, M), cols), preferred_element_type=f32)
            if i >= 2:
                out_copy(i - 2).wait()
            out_v[i % 2] = (g * a + (1.0 - g) * b).astype(bf16)
            out_copy(i).start()
        out_copy(len(blocks) - 2).wait()
        out_copy(len(blocks) - 1).wait()

    pl.run_scoped(phase23, pltpu.VMEM((NS, BQ, S), f32), pltpu.VMEM((H, S // 2, D), u32), pltpu.VMEM((2, RO, CO), bf16))


@jax.jit
def pallas_gated_mix__compressed_kv_cla__sliding_local_dilated__prompt_kernel(
    A_x, A_c_kv, A_w_q, A_w_uk, A_w_uv, A_w_o, B_x, B_wqkv, B_wo, gate_w,
):
    del B_x
    any_spec = pl.BlockSpec(memory_space=pl.ANY)
    out = pl.pallas_call(
        _kernel,
        out_shape=jax.ShapeDtypeStruct((S, M), bf16),
        in_specs=[any_spec] * 9,
        out_specs=any_spec,
        scratch_shapes=[
            pltpu.VMEM((S // 2, M), u32), pltpu.VMEM((S // 2, DC), u32),
            pltpu.VMEM((M // 8, 8 * WP, D), u32), pltpu.VMEM((DC // 8, 8 * WP, D), u32),
            pltpu.VMEM((DC // 8, 8 * WP, D), u32),
            pltpu.VMEM((H * D // 2, M), u32), pltpu.VMEM((1, M), bf16), pltpu.VMEM((M // 2, M), u32),
            pltpu.VMEM((S // 2, M), u32),
            pltpu.VMEM((LT, S, 128), f32), pltpu.VMEM((LT, S + PAD, 128), f32), pltpu.VMEM((LT, S + PAD, 128), f32),
            pltpu.VMEM((M // 2, 2 * D), u32), pltpu.VMEM((DC // 2, 4 * D), u32),
            pltpu.VMEM((2, S // 2, D), u32), pltpu.VMEM((2, S // 2, D), u32), pltpu.VMEM((2, S // 2, D), u32),
            pltpu.SMEM((1,), jnp.int32), pltpu.SemaphoreType.DMA((S // RB + 10 + M // 128,)), pltpu.SemaphoreType.DMA((2,)),
        ],
        compiler_params=pltpu.CompilerParams(vmem_limit_bytes=120 * 1024 * 1024),
    )(
        A_x.reshape(S, M), A_c_kv.reshape(S, DC), A_w_q.reshape(M // 8, 8, H, D), A_w_uk.reshape(DC // 8, 8, H, D),
        A_w_uv.reshape(DC // 8, 8, H, D), A_w_o.reshape(H * D, M), B_wqkv, B_wo, gate_w.reshape(1, M),
    )
    return out.reshape(1, S, M)
```

```python
import functools

import jax
import jax.numpy as jnp
from jax import lax
import jax.experimental.pallas as pl
import jax.experimental.pallas.tpu as pltpu

S = 2048
M = 1024
H = 32
D = 128
DC = 512
DH = 32
W = 8
DIL = 2
PAD = 16
PITCH = DH + 1
BQ = 256
NQ = S // BQ
NP = H // 2
RB = 256
NB = 256
RP = 256
RI = 16
RL = S // NP
RO = 2048
CW = 256
DIAG = 1
NS = 2
LAG = 1
PINP = 3
PINL = 1
PINW = 0
WP = H // 2 + 1
CO = 512
CUT = 1792
LS = 112
ALL = slice(None)
LT = M // 128
LOG2E = 1.4426950408889634
NEG = -1e9
NT = (((1,), (1,)), ((), ()))
f32, bf16, u32 = jnp.float32, jnp.bfloat16, jnp.uint32


def _run(*lists):
    items = []
    for k, l in enumerate(lists):
        items += [((i + 0.5) / len(l), k, f) for i, f in enumerate(l)]
    items.sort(key=lambda t: (t[0], t[1]))
    for _, _, f in items:
        f()


def _unpack(u):
    lo = lax.bitcast_convert_type(u << 16, f32)
    hi = lax.bitcast_convert_type(u & jnp.uint32(0xFFFF0000), f32)
    return lo, hi


def _half(rows):
    if isinstance(rows, slice):
        return slice(rows.start // 2, rows.stop // 2)
    start = rows.start // 2
    return pl.ds(start if isinstance(start, int) else pl.multiple_of(start, 8), rows.size // 2)


def _ld(ref, rows, cols=slice(None)):
    return pltpu.bitcast(ref[_half(rows), cols], bf16)


def _st(ref, rows, cols, val):
    ref[_half(rows), cols] = pltpu.bitcast(val, u32)


def _lane_tiles(x):
    return [x[:, t * 128:(t + 1) * 128] for t in range(x.shape[1] // 128)]


def _kernel(x_hbm, ckv_hbm, wq_hbm, wuk_hbm, wuv_hbm, wo_hbm, wqkv_hbm, wob_hbm, gw_hbm, out_hbm,
            x_v, ckv_v, wq_v, wuk_v, wuv_v, wo_v, gw_v, wobp_v, ob_v, qb_v, kb_v, vb_v,
            wa_v, wb_v, q_v, k_v, v_v, zero_s, sem, osem):
    zero_s[0] = 0
    toks = []

    def pin(lhs):
        if not toks:
            return lhs
        tok = functools.reduce(lambda a, b: a | b, toks)
        toks.clear()
        never = (lax.broadcasted_iota(jnp.int32, (8, 128), 1) + zero_s[0]) < 0
        head = pltpu.bitcast(lhs[0:16, 0:128], u32)
        head = pltpu.bitcast(jnp.where(never, tok, head), bf16)
        top = head if lhs.shape[1] == 128 else jnp.concatenate([head, lhs[0:16, 128:]], axis=1)
        return jnp.concatenate([top, lhs[16:]], axis=0)

    def cp(src, dst, i):
        return pltpu.make_async_copy(src, dst, sem.at[i])

    NX = S // RB
    HR = RB // 2
    x_cp = [cp(x_hbm.bitcast(u32).at[i * HR:(i + 1) * HR, :], x_v.at[i * HR:(i + 1) * HR, :], i) for i in range(NX)]
    gw_cp = cp(gw_hbm, gw_v, NX + 4)
    ckv_cp = cp(ckv_hbm.bitcast(u32), ckv_v, NX + 5)
    def w_cps(src, dst, i):
        return [cp(src.bitcast(u32).at[:, c], dst.at[:, c * WP:c * WP + NP, :], i) for c in range(8)]
    wq_cp = w_cps(wq_hbm, wq_v, NX + 6)
    wuk_cp = w_cps(wuk_hbm, wuk_v, NX + 7)
    wuv_cp = w_cps(wuv_hbm, wuv_v, NX + 8)
    wo_cp = cp(wo_hbm.bitcast(u32), wo_v, NX + 9)

    def wprep_steps(j, tok=False):
        def one(src, dst, r0, n, c0, c1):
            def f():
                u = [src[g, pl.ds(j, 8, stride=WP), :] for g in range(r0 // 8, (r0 + n) // 8)]
                lo, hi = _unpack(jnp.concatenate(u, axis=0))
                lo, hi = lo.astype(bf16), hi.astype(bf16)
                _st(dst, slice(r0, r0 + n), slice(c0, c0 + D), lo)
                _st(dst, slice(r0, r0 + n), slice(c1, c1 + D), hi)
                if PINW and tok:
                    toks.extend(pltpu.bitcast(x[i:i + 16], u32) for x in (lo, hi) for i in range(0, n, 16))
            return f
        n = 256
        return ([one(wq_v, wa_v, r0, n, 0, D) for r0 in range(0, M, n)]
                + [one(wuk_v, wb_v, r0, n, 0, D) for r0 in range(0, DC, n)]
                + [one(wuv_v, wb_v, r0, n, 2 * D, 3 * D) for r0 in range(0, DC, n)])

    def aproj_steps(base, rows):
        def kv_piece(r0):
            def f():
                r = slice(base + r0, base + r0 + RP)
                y = jnp.dot(pin(_ld(ckv_v, r)), _ld(wb_v, slice(0, DC)), preferred_element_type=f32).astype(bf16)
                _st(k_v.at[0], r, ALL, y[:, 0 * D:1 * D])
                _st(k_v.at[1], r, ALL, y[:, 1 * D:2 * D])
                _st(v_v.at[0], r, ALL, y[:, 2 * D:3 * D])
                _st(v_v.at[1], r, ALL, y[:, 3 * D:4 * D])
            return f

        def q_piece(r0):
            def f():
                r = slice(base + r0, base + r0 + RP)
                y = jnp.dot(pin(_ld(x_v, r)), _ld(wa_v, slice(0, M)), preferred_element_type=f32)
                y = (y * (D ** -0.5 * LOG2E)).astype(bf16)
                _st(q_v.at[0], r, ALL, y[:, :D])
                _st(q_v.at[1], r, ALL, y[:, D:])
            return f
        return [kv_piece(r0) for r0 in range(0, rows, RP)] + [q_piece(r0) for r0 in range(0, rows, RP)]

    def local_steps(r0, rows):
        def block(ib):
            def f():
                r = r0 + ib * RI
                qt = [qb_v[t, pl.ds(r, RI), :] for t in range(LT)]
                pos = r + lax.broadcasted_iota(jnp.int32, (RI, 128), 0)
                logits = []
                for w in range(W):
                    acc = None
                    for t in range(LT):
                        pr = qt[t] * kb_v[t, pl.ds(r + PAD - w * DIL, RI), :]
                        acc = pr if acc is None else acc + pr
                    acc = acc + pltpu.roll(acc, 64, 1)
                    acc = acc + pltpu.roll(acc, 32, 1)
                    if w > 0:
                        acc = jnp.where(pos >= w * DIL, acc, NEG * LOG2E)
                    logits.append(acc)
                m = functools.reduce(jnp.maximum, logits)
                ps = [jnp.exp2(l - m) for l in logits]
                inv = 1.0 / functools.reduce(lambda a, b: a + b, ps)
                ps = [p * inv for p in ps]
                for t in range(LT):
                    o = None
                    for w in range(W):
                        term = ps[w] * vb_v[t, pl.ds(r + PAD - w * DIL, RI), :]
                        o = term if o is None else o + term
                    ob = o.astype(bf16)
                    _st(ob_v, pl.ds(r, RI), slice(t * 128, (t + 1) * 128), ob)
                    if PINL:
                        toks.append(pltpu.bitcast(ob[0:16], u32))
            return f
        return [block(ib) for ib in range(rows // RI)]

    def phase1(wqkv_v, wob_v, wt_v, wtp_v):
        def wcols(c0, n, i):
            return cp(wqkv_hbm.at[:, c0:c0 + n], wqkv_v.at[:, c0:c0 + n], i)
        wk_cp = [wcols(M + t * 128, 128, NX + 10 + t) for t in range(LT)]
        wqkv_cp = [wcols(0, M, NX), None, wcols(2 * M, M, NX + 2)]
        wob_cp = [cp(wob_hbm.bitcast(u32).at[:, t * 128:(t + 1) * 128], wob_v.at[t], NX + 3) for t in range(LT)]
        third = wob_cp + wq_cp + wuk_cp + wuv_cp + [ckv_cp, wo_cp, gw_cp]
        OR = '1'
        if OR == '0':
            lst = wk_cp + [x_cp[0], wqkv_cp[2]] + x_cp[1:] + [wqkv_cp[0]]
        elif OR == '1':
            lst = wk_cp + [x_cp[0], x_cp[1], wqkv_cp[2]] + x_cp[2:] + [wqkv_cp[0]]
        else:
            lst = [x_cp[0]] + wk_cp + [x_cp[1], wqkv_cp[2]] + x_cp[2:] + [wqkv_cp[0]]
        for c in lst:
            c.start()
        T3 = 3

        def prep_steps(p):
            def tr(t):
                def f():
                    if p == 1:
                        wk_cp[t].wait()
                    elif t == 0:
                        wqkv_cp[p].wait()
                    blk_t = wqkv_v[:, p * M + t * 128:p * M + (t + 1) * 128].astype(f32).T
                    for hl in range(128 // DH):
                        r = (t * (128 // DH) + hl) * PITCH
                        for mt in range(LT):
                            wt_v[mt, r:r + DH, :] = blk_t[hl * DH:(hl + 1) * DH, mt * 128:(mt + 1) * 128]
                return f

            def perm(d0):
                def f():
                    for dh in range(d0, d0 + 4):
                        for mt in range(LT):
                            rows = wt_v[mt, pl.ds(dh, H, stride=PITCH), :]
                            rows = rows.astype(bf16)
                            _st(wtp_v, slice(p * M + dh * H, p * M + (dh + 1) * H), slice(mt * 128, (mt + 1) * 128), rows)
                            if PINP and p != 1:
                                toks.extend(pltpu.bitcast(rows[i:i + 16], u32) for i in range(0, H, 16))
                return f
            return [tr(t) for t in range(LT)] + [perm(d0) for d0 in range(0, DH, 4)]

        def proj_steps(p):
            def piece(i, c0):
                def f():
                    if p == 1 and c0 == 0:
                        x_cp[i].wait()
                        if i == T3:
                            for c in third:
                                c.start()
                    r0 = i * RB
                    y = lax.dot_general(pin(_ld(x_v, slice(r0, r0 + RB))), _ld(wtp_v, slice(p * M + c0, p * M + c0 + NB)), NT,
                                        preferred_element_type=f32)
                    if p == 0:
                        y = y * (DH ** -0.5 * LOG2E)
                    for t, yt in enumerate(_lane_tiles(y)):
                        if p == 0:
                            qb_v[c0 // 128 + t, r0:r0 + RB, :] = yt
                        elif p == 1:
                            kb_v[c0 // 128 + t, PAD + r0:PAD + r0 + RB, :] = yt
                        else:
                            vb_v[c0 // 128 + t, PAD + r0:PAD + r0 + RB, :] = yt
                return f
            return [piece(i, c0) for i in range(NX) for c0 in range(0, M, NB)]

        def wob_steps():
            def one(j):
                def f():
                    if j == 0:
                        for c in wob_cp:
                            c.wait()
                    for t in range(LT):
                        lo, hi = _unpack(wob_v[t, pl.ds(j, H, stride=DH // 2), :])
                        rows = jnp.concatenate([lo, hi], axis=0).astype(bf16)
                        _st(wobp_v, slice(2 * j * H, (2 * j + 2) * H), slice(t * 128, (t + 1) * 128), rows)
                        if PINP & 2:
                            toks.extend(pltpu.bitcast(rows[i:i + 16], u32) for i in range(0, 2 * H, 16))
                return f
            return [one(j) for j in range(DH // 2)]

        kb_v[:, 0:PAD, :] = jnp.zeros((LT, PAD, 128), f32)
        vb_v[:, 0:PAD, :] = jnp.zeros((LT, PAD, 128), f32)
        pk = prep_steps(1)
        _run(pk[:LT])
        _run(pk[LT:])
        pj = proj_steps(1)
        pv = prep_steps(2)
        KS = 2
        per = len(pj) // NX
        for i in range(NX):
            if i < KS:
                _run(pj[i * per:(i + 1) * per])
            else:
                n0, n1 = [len(pv) * (ii - KS) // (NX - KS) for ii in (i, i + 1)]
                _run(pj[i * per:(i + 1) * per], pv[n0:n1])
        _run(proj_steps(2), prep_steps(0))

        def waits():
            for c in wq_cp + wuk_cp + wuv_cp + [ckv_cp]:
                c.wait()
        _run(proj_steps(0), wob_steps() + [waits] + wprep_steps(0))
        toks.clear()
        _run(aproj_steps(CUT, S - CUT))

    pl.run_scoped(phase1, pltpu.VMEM((M, 3 * M), bf16), pltpu.VMEM((LT, M // 2, 128), u32),
                  pltpu.VMEM((LT, H * PITCH, 128), f32), pltpu.VMEM((3 * M // 2, M), u32))

    def phase23(s_v, ctx_v, out_v):
        HB = BQ // 2

        def attn_steps(j):
            orders = '76543210,76543210'.split(',')
            tasks = [(e, int(ch)) for e in range(2) for ch in orders[e]]
            rowmax = {}

            def segments(qi):
                segs, k0 = [], 0
                while k0 < qi * BQ:
                    wd = CW if k0 + CW <= qi * BQ else BQ
                    segs.append((k0, wd))
                    k0 += wd
                return segs

            def p1_steps(n):
                e, qi = tasks[n]
                sb = s_v.at[n % NS]
                r0 = qi * BQ
                state = {"m": None}

                def upd(m, s):
                    for x in _lane_tiles(s):
                        m = x if m is None else jnp.maximum(m, x)
                    return m

                def full(k0, wd):
                    def f():
                        s = lax.dot_general(pin(_ld(q_v.at[e], slice(r0, r0 + BQ))), _ld(k_v.at[e], slice(k0, k0 + wd)), NT,
                                            preferred_element_type=f32)
                        sb[:, k0:k0 + wd] = s
                        state["m"] = upd(state["m"], s)
                    return f

                def diag():
                    neg = NEG * D ** -0.5 * LOG2E
                    if DIAG == 0:
                        tri = (lax.broadcasted_iota(jnp.int32, (BQ, BQ), 1)
                               <= lax.broadcasted_iota(jnp.int32, (BQ, BQ), 0))
                        s = lax.dot_general(_ld(q_v.at[e], slice(r0, r0 + BQ)), _ld(k_v.at[e], slice(r0, r0 + BQ)), NT,
                                            preferred_element_type=f32)
                        s = jnp.where(tri, s, neg)
                        sb[:, r0:r0 + BQ] = s
                        md = upd(None, s)
                    else:
                        tri = (lax.broadcasted_iota(jnp.int32, (HB, HB), 1)
                               <= lax.broadcasted_iota(jnp.int32, (HB, HB), 0))
                        sa = lax.dot_general(_ld(q_v.at[e], slice(r0, r0 + BQ)), _ld(k_v.at[e], slice(r0, r0 + HB)), NT,
                                             preferred_element_type=f32)
                        sa = jnp.concatenate([jnp.where(tri, sa[:HB], neg), sa[HB:]], axis=0)
                        sc = lax.dot_general(_ld(q_v.at[e], slice(r0 + HB, r0 + BQ)), _ld(k_v.at[e], slice(r0 + HB, r0 + BQ)), NT,
                                             preferred_element_type=f32)
                        sc = jnp.where(tri, sc, neg)
                        sb[:, r0:r0 + HB] = sa
                        sb[HB:BQ, r0 + HB:r0 + BQ] = sc
                        md = jnp.concatenate([sa[:HB], jnp.maximum(sa[HB:], sc)], axis=0)
                    m = md if state["m"] is None else jnp.maximum(state["m"], md)
                    rowmax[n] = jnp.max(m, axis=1, keepdims=True)
                return [full(*sg) for sg in segments(qi)] + [diag]

            def p2_steps(n):
                e, qi = tasks[n]
                sb = s_v.at[n % NS]
                r0 = qi * BQ
                state = {"l": None, "acc": None}

                def lsum(l, p):
                    t = None
                    for x in _lane_tiles(p):
                        t = x if t is None else t + x
                    return t if l is None else l + t

                def full(k0, wd):
                    def f():
                        p = jnp.exp2(sb[:, k0:k0 + wd] - rowmax[n])
                        state["l"] = lsum(state["l"], p)
                        o = jnp.dot(p.astype(bf16), _ld(v_v.at[e], slice(k0, k0 + wd)), preferred_element_type=f32)
                        state["acc"] = o if state["acc"] is None else state["acc"] + o
                    return f

                def diag():
                    m = rowmax[n]
                    if DIAG == 0:
                        p = jnp.exp2(sb[:, r0:r0 + BQ] - m)
                        l = lsum(None, p)
                        acc = jnp.dot(p.astype(bf16), _ld(v_v.at[e], slice(r0, r0 + BQ)), preferred_element_type=f32)
                    else:
                        pa = jnp.exp2(sb[:, r0:r0 + HB] - m)
                        pc = jnp.exp2(sb[HB:BQ, r0 + HB:r0 + BQ] - m[HB:])
                        oa = jnp.dot(pa.astype(bf16), _ld(v_v.at[e], slice(r0, r0 + HB)), preferred_element_type=f32)
                        oc = jnp.dot(pc.astype(bf16), _ld(v_v.at[e], slice(r0 + HB, r0 + BQ)), preferred_element_type=f32)
                        l = jnp.concatenate([pa[:HB], pa[HB:] + pc], axis=0)
                        acc = jnp.concatenate([oa[:HB], oa[HB:] + oc], axis=0)
                    if state["l"] is not None:
                        l = l + state["l"]
                        acc = acc + state["acc"]
                    l = jnp.sum(l, axis=1, keepdims=True)
                    inv = pl.reciprocal(l, approx=True)
                    inv = inv * (2.0 - l * inv)
                    _st(ctx_v.at[2 * j + e], slice(r0, r0 + BQ), ALL, (acc * inv).astype(bf16))
                return [full(*sg) for sg in segments(qi)] + [diag]

            sa = [(n, f) for n in range(len(tasks)) for f in p1_steps(n)]
            sb_ = [(n, f) for n in range(len(tasks)) for f in p2_steps(n)]
            end_a = {n: i + 1 for i, (n, _) in enumerate(sa)}
            end_b = {n: i + 1 for i, (n, _) in enumerate(sb_)}
            steps, ia, ib, last = [], 0, 0, "b"
            while ia < len(sa) or ib < len(sb_):
                can_a = ia < len(sa) and (sa[ia][0] < NS or ib >= end_b[sa[ia][0] - NS])
                can_b = ib < len(sb_) and (ia >= min(end_a[sb_[ib][0]] + LAG, len(sa)) or not can_a)
                if can_a and (last == "b" or not can_b):
                    steps.append(sa[ia][1])
                    ia, last = ia + 1, "a"
                else:
                    assert ia >= end_a[sb_[ib][0]]
                    steps.append(sb_[ib][1])
                    ib, last = ib + 1, "b"
            n_hi = max(n for n, (e, qi) in enumerate(tasks) if qi * BQ >= CUT)
            cut = steps.index(sb_[end_b[n_hi] - 1][1]) + 1
            return steps[:cut], steps[cut:]

        def pair(j, last):
            if CUT > 0:
                _run(aproj_steps(0, CUT), local_steps(pl.multiple_of(j * RL, RL), LS))
                toks.clear()
            head, tail = attn_steps(j)
            _run(head)
            if last:
                _run(tail, local_steps(j * RL + LS, RL - LS))
            else:
                _run(tail, wprep_steps(j + 1) + aproj_steps(CUT, S - CUT),
                     local_steps(pl.multiple_of(j * RL + LS, RI), RL - LS))
            toks.clear()

        def pair_body(j, c):
            pair(j, False)
            return c

        lax.fori_loop(0, NP - 1, pair_body, 0)
        pair(NP - 1, True)

        gw_cp.wait()
        wo_cp.wait()
        gw = gw_v[...].astype(f32).reshape(1, M)
        blocks = [tuple(int(v) for v in b.split(':')) for b in '0:2048:0:512,0:2048:512:384,0:1024:896:128,1024:1024:896:128'.split(',')]

        def out_copy(i):
            r, nr, c, nc = blocks[i]
            return pltpu.make_async_copy(out_v.at[i % 2, 0:nr, 0:nc], out_hbm.at[r:r + nr, c:c + nc], osem.at[i % 2])

        g = jax.nn.sigmoid(jnp.sum(_ld(x_v, slice(0, S)).astype(f32) * gw, axis=1, keepdims=True))
        for i, (r, nr, c, nc) in enumerate(blocks):
            rows, cols = slice(r, r + nr), slice(c, c + nc)
            a = None
            for h in range(H):
                t = jnp.dot(_ld(ctx_v.at[h], rows), _ld(wo_v, slice(h * D, (h + 1) * D), cols),
                            preferred_element_type=f32)
                a = t if a is None else a + t
            b = jnp.dot(_ld(ob_v, rows), _ld(wobp_v, slice(0, M), cols), preferred_element_type=f32)
            if i >= 2:
                out_copy(i - 2).wait()
            gr = g[r:r + nr]
            out_v[i % 2, 0:nr, 0:nc] = (gr * a + (1.0 - gr) * b).astype(bf16)
            out_copy(i).start()
        out_copy(len(blocks) - 2).wait()
        out_copy(len(blocks) - 1).wait()

    pl.run_scoped(phase23, pltpu.VMEM((NS, BQ, S), f32), pltpu.VMEM((H, S // 2, D), u32), pltpu.VMEM((2, S, 512), bf16))


@jax.jit
def pallas_gated_mix__compressed_kv_cla__sliding_local_dilated__prompt_kernel(
    A_x, A_c_kv, A_w_q, A_w_uk, A_w_uv, A_w_o, B_x, B_wqkv, B_wo, gate_w,
):
    del B_x
    any_spec = pl.BlockSpec(memory_space=pl.ANY)
    out = pl.pallas_call(
        _kernel,
        out_shape=jax.ShapeDtypeStruct((S, M), bf16),
        in_specs=[any_spec] * 9,
        out_specs=any_spec,
        scratch_shapes=[
            pltpu.VMEM((S // 2, M), u32), pltpu.VMEM((S // 2, DC), u32),
            pltpu.VMEM((M // 8, 8 * WP, D), u32), pltpu.VMEM((DC // 8, 8 * WP, D), u32),
            pltpu.VMEM((DC // 8, 8 * WP, D), u32),
            pltpu.VMEM((H * D // 2, M), u32), pltpu.VMEM((M,), bf16), pltpu.VMEM((M // 2, M), u32),
            pltpu.VMEM((S // 2, M), u32),
            pltpu.VMEM((LT, S, 128), f32), pltpu.VMEM((LT, S + PAD, 128), f32), pltpu.VMEM((LT, S + PAD, 128), f32),
            pltpu.VMEM((M // 2, 2 * D), u32), pltpu.VMEM((DC // 2, 4 * D), u32),
            pltpu.VMEM((2, S // 2, D), u32), pltpu.VMEM((2, S // 2, D), u32), pltpu.VMEM((2, S // 2, D), u32),
            pltpu.SMEM((1,), jnp.int32), pltpu.SemaphoreType.DMA((S // RB + 10 + M // 128,)), pltpu.SemaphoreType.DMA((2,)),
        ],
        compiler_params=pltpu.CompilerParams(vmem_limit_bytes=126 * 1024 * 1024),
    )(
        A_x.reshape(S, M), A_c_kv.reshape(S, DC), A_w_q.reshape(M // 8, 8, H, D), A_w_uk.reshape(DC // 8, 8, H, D),
        A_w_uv.reshape(DC // 8, 8, H, D), A_w_o.reshape(H * D, M), B_wqkv, B_wo, gate_w,
    )
    return out.reshape(1, S, M)
```

```python
import functools

import jax
import jax.numpy as jnp
from jax import lax
import jax.experimental.pallas as pl
import jax.experimental.pallas.tpu as pltpu

S = 2048
M = 1024
H = 32
D = 128
DC = 512
DH = 32
W = 8
DIL = 2
PAD = 16
PITCH = DH + 1
BQ = 256
NQ = S // BQ
NP = H // 2
RB = 256
NB = 256
RP = 256
RI = 16
RL = S // NP
RO = 2048
CW = 256
DIAG = 1
NS = 2
LAG = 1
PINP = 3
PINL = 1
PINW = 0
WP = H // 2 + 1
CO = 512
CUT = 1792
LS = 112
R0 = 512
KS = 4
ALL = slice(None)
LT = M // 128
LOG2E = 1.4426950408889634
NEG = -1e9
NT = (((1,), (1,)), ((), ()))
f32, bf16, u32 = jnp.float32, jnp.bfloat16, jnp.uint32


def _run(*lists):
    items = []
    for k, l in enumerate(lists):
        items += [((i + 0.5) / len(l), k, f) for i, f in enumerate(l)]
    items.sort(key=lambda t: (t[0], t[1]))
    for _, _, f in items:
        f()


def _unpack(u):
    lo = lax.bitcast_convert_type(u << 16, f32)
    hi = lax.bitcast_convert_type(u & jnp.uint32(0xFFFF0000), f32)
    return lo, hi


def _half(rows):
    if isinstance(rows, slice):
        return slice(rows.start // 2, rows.stop // 2)
    start = rows.start // 2
    return pl.ds(start if isinstance(start, int) else pl.multiple_of(start, 8), rows.size // 2)


def _ld(ref, rows, cols=slice(None)):
    return pltpu.bitcast(ref[_half(rows), cols], bf16)


def _st(ref, rows, cols, val):
    ref[_half(rows), cols] = pltpu.bitcast(val, u32)


def _lane_tiles(x):
    return [x[:, t * 128:(t + 1) * 128] for t in range(x.shape[1] // 128)]


def _kernel(x_hbm, ckv_hbm, wq_hbm, wuk_hbm, wuv_hbm, wo_hbm, wqkv_hbm, wob_hbm, gw_hbm, out_hbm,
            x_v, ckv_v, wq_v, wuk_v, wuv_v, wo_v, gw_v, wobp_v, ob_v, qb_v, kb_v, vb_v,
            wa_v, wb_v, q_v, k_v, v_v, zero_s, sem, osem):
    zero_s[0] = 0
    toks = []

    def pin(lhs):
        if not toks:
            return lhs
        tok = functools.reduce(lambda a, b: a | b, toks)
        toks.clear()
        never = (lax.broadcasted_iota(jnp.int32, (8, 128), 1) + zero_s[0]) < 0
        head = pltpu.bitcast(lhs[0:16, 0:128], u32)
        head = pltpu.bitcast(jnp.where(never, tok, head), bf16)
        top = head if lhs.shape[1] == 128 else jnp.concatenate([head, lhs[0:16, 128:]], axis=1)
        return jnp.concatenate([top, lhs[16:]], axis=0)

    def cp(src, dst, i):
        return pltpu.make_async_copy(src, dst, sem.at[i])

    NX = S // RB
    HR = RB // 2
    x_cp = [cp(x_hbm.bitcast(u32).at[i * HR:(i + 1) * HR, :], x_v.at[i * HR:(i + 1) * HR, :], i) for i in range(NX)]
    gw_cp = cp(gw_hbm, gw_v, NX + 4)
    ckv_cp = cp(ckv_hbm.bitcast(u32), ckv_v, NX + 5)
    def w_cps(src, dst, i):
        return [cp(src.bitcast(u32).at[:, c], dst.at[:, c * WP:c * WP + NP, :], i) for c in range(8)]
    wq_cp = w_cps(wq_hbm, wq_v, NX + 6)
    wuk_cp = w_cps(wuk_hbm, wuk_v, NX + 7)
    wuv_cp = w_cps(wuv_hbm, wuv_v, NX + 8)
    wo_cp = cp(wo_hbm.bitcast(u32), wo_v, NX + 9)

    def wprep_steps(j, tok=False):
        def one(src, dst, r0, n, c0, c1):
            def f():
                u = [src[g, pl.ds(j, 8, stride=WP), :] for g in range(r0 // 8, (r0 + n) // 8)]
                lo, hi = _unpack(jnp.concatenate(u, axis=0))
                lo, hi = lo.astype(bf16), hi.astype(bf16)
                _st(dst, slice(r0, r0 + n), slice(c0, c0 + D), lo)
                _st(dst, slice(r0, r0 + n), slice(c1, c1 + D), hi)
                if tok:
                    toks.extend(pltpu.bitcast(x[i:i + 16], u32) for x in (lo, hi) for i in range(0, n, 16))
            return f
        n = 256
        return ([one(wq_v, wa_v, r0, n, 0, D) for r0 in range(0, M, n)]
                + [one(wuk_v, wb_v, r0, n, 0, D) for r0 in range(0, DC, n)]
                + [one(wuv_v, wb_v, r0, n, 2 * D, 3 * D) for r0 in range(0, DC, n)])

    def aproj_steps(base, rows):
        def kv_piece(r0):
            def f():
                r = slice(base + r0, base + r0 + RP)
                y = jnp.dot(pin(_ld(ckv_v, r)), _ld(wb_v, slice(0, DC)), preferred_element_type=f32).astype(bf16)
                _st(k_v.at[0], r, ALL, y[:, 0 * D:1 * D])
                _st(k_v.at[1], r, ALL, y[:, 1 * D:2 * D])
                _st(v_v.at[0], r, ALL, y[:, 2 * D:3 * D])
                _st(v_v.at[1], r, ALL, y[:, 3 * D:4 * D])
            return f

        def q_piece(r0):
            def f():
                r = slice(base + r0, base + r0 + RP)
                y = jnp.dot(pin(_ld(x_v, r)), _ld(wa_v, slice(0, M)), preferred_element_type=f32)
                y = (y * (D ** -0.5 * LOG2E)).astype(bf16)
                _st(q_v.at[0], r, ALL, y[:, :D])
                _st(q_v.at[1], r, ALL, y[:, D:])
            return f
        return [kv_piece(r0) for r0 in range(0, rows, RP)] + [q_piece(r0) for r0 in range(0, rows, RP)]

    def local_steps(r0, rows):
        def block(ib):
            def f():
                r = r0 + ib * RI
                qt = [qb_v[t, pl.ds(r, RI), :] for t in range(LT)]
                pos = r + lax.broadcasted_iota(jnp.int32, (RI, 128), 0)
                logits = []
                for w in range(W):
                    acc = None
                    for t in range(LT):
                        pr = qt[t] * kb_v[t, pl.ds(r + PAD - w * DIL, RI), :]
                        acc = pr if acc is None else acc + pr
                    acc = acc + pltpu.roll(acc, 64, 1)
                    acc = acc + pltpu.roll(acc, 32, 1)
                    if w > 0:
                        acc = jnp.where(pos >= w * DIL, acc, NEG * LOG2E)
                    logits.append(acc)
                m = functools.reduce(jnp.maximum, logits)
                ps = [jnp.exp2(l - m) for l in logits]
                inv = 1.0 / functools.reduce(lambda a, b: a + b, ps)
                ps = [p * inv for p in ps]
                for t in range(LT):
                    o = None
                    for w in range(W):
                        term = ps[w] * vb_v[t, pl.ds(r + PAD - w * DIL, RI), :]
                        o = term if o is None else o + term
                    ob = o.astype(bf16)
                    _st(ob_v, pl.ds(r, RI), slice(t * 128, (t + 1) * 128), ob)
                    if PINL:
                        toks.append(pltpu.bitcast(ob[0:16], u32))
            return f
        return [block(ib) for ib in range(rows // RI)]

    def phase1(wqkv_v, wob_v, wt_v, wtp_v):
        def wcols(c0, n, i):
            return cp(wqkv_hbm.at[:, c0:c0 + n], wqkv_v.at[:, c0:c0 + n], i)
        wk_cp = [cp(wqkv_hbm.at[t * 128:(t + 1) * 128, M:2 * M], wqkv_v.at[t * 128:(t + 1) * 128, M:2 * M], NX + 10 + t)
                 for t in range(LT)]
        wqkv_cp = [wcols(0, M, NX), None, wcols(2 * M, M, NX + 2)]
        wob_cp = [cp(wob_hbm.bitcast(u32).at[:, t * 128:(t + 1) * 128], wob_v.at[t], NX + 3) for t in range(LT)]
        third = wob_cp + wq_cp + wuk_cp + wuv_cp + [ckv_cp, wo_cp, gw_cp]
        N0 = R0 // RB
        for c in x_cp[:N0] + wk_cp + x_cp[N0:] + [wqkv_cp[2], wqkv_cp[0]]:
            c.start()

        def prep_steps(p):
            def tr(mt):
                def f():
                    if p == 1:
                        wk_cp[mt].wait()
                    blk_t = wqkv_v[mt * 128:(mt + 1) * 128, p * M:(p + 1) * M].astype(f32).T
                    for h in range(H):
                        wt_v[mt, h * PITCH:h * PITCH + DH, :] = blk_t[h * DH:(h + 1) * DH, :]
                return f

            def perm(mt):
                def f():
                    for dh in range(DH):
                        rows = wt_v[mt, pl.ds(dh, H, stride=PITCH), :].astype(bf16)
                        _st(wtp_v, slice(p * M + dh * H, p * M + (dh + 1) * H), slice(mt * 128, (mt + 1) * 128), rows)
                        if PINP and p != 1:
                            toks.extend(pltpu.bitcast(rows[i:i + 16], u32) for i in range(0, H, 16))
                return f
            return [g(mt) for mt in range(LT) for g in (tr, perm)]

        def proj_steps(p):
            def piece(i, c0):
                def f():
                    if p == 1 and c0 == 0 and i == N0:
                        for c in x_cp[N0:KS]:
                            c.wait()
                    r0 = i * RB
                    y = lax.dot_general(pin(_ld(x_v, slice(r0, r0 + RB))), _ld(wtp_v, slice(p * M + c0, p * M + c0 + NB)), NT,
                                        preferred_element_type=f32)
                    if p == 0:
                        y = y * (DH ** -0.5 * LOG2E)
                    for t, yt in enumerate(_lane_tiles(y)):
                        if p == 0:
                            qb_v[c0 // 128 + t, r0:r0 + RB, :] = yt
                        elif p == 1:
                            kb_v[c0 // 128 + t, PAD + r0:PAD + r0 + RB, :] = yt
                        else:
                            vb_v[c0 // 128 + t, PAD + r0:PAD + r0 + RB, :] = yt
                return f
            return [piece(i, c0) for i in range(N0 if p == 1 else 0, NX) for c0 in range(0, M, NB)]

        def wob_steps():
            def one(j):
                def f():
                    for t in range(LT):
                        lo, hi = _unpack(wob_v[t, pl.ds(j, H, stride=DH // 2), :])
                        rows = jnp.concatenate([lo, hi], axis=0).astype(bf16)
                        _st(wobp_v, slice(2 * j * H, (2 * j + 2) * H), slice(t * 128, (t + 1) * 128), rows)
                        if PINP & 2:
                            toks.extend(pltpu.bitcast(rows[i:i + 16], u32) for i in range(0, 2 * H, 16))
                return f
            return [one(j) for j in range(DH // 2)]

        kb_v[:, 0:PAD, :] = jnp.zeros((LT, PAD, 128), f32)
        vb_v[:, 0:PAD, :] = jnp.zeros((LT, PAD, 128), f32)
        pk = prep_steps(1)
        for c in x_cp[:N0]:
            c.wait()
        y = None
        pk[0]()
        pk[1]()
        for mt in range(LT):
            for f in pk[2 * mt + 2:2 * mt + 4]:
                f()
            cols = slice(mt * 128, (mt + 1) * 128)
            t = lax.dot_general(_ld(x_v, slice(0, R0), cols), _ld(wtp_v, slice(M, 2 * M), cols), NT,
                                preferred_element_type=f32)
            y = t if y is None else y + t
        for t, yt in enumerate(_lane_tiles(y)):
            kb_v[t, PAD:PAD + R0, :] = yt
        pj = proj_steps(1)
        pv = prep_steps(2)
        per = M // NB
        pj = [None] * (N0 * per) + pj
        for i in range(N0, NX):
            if i < KS:
                _run(pj[i * per:(i + 1) * per])
            else:
                if i == KS:
                    for c in x_cp[KS:] + [wqkv_cp[2], wqkv_cp[0]]:
                        c.wait()
                    for c in third:
                        c.start()
                n0, n1 = [len(pv) * (ii - KS) // (NX - KS) for ii in (i, i + 1)]
                _run(pj[i * per:(i + 1) * per], pv[n0:n1])
        _run(proj_steps(2), prep_steps(0))

        def waits():
            for c in wob_cp + wq_cp + wuk_cp + wuv_cp + [ckv_cp]:
                c.wait()
        _run(proj_steps(0), [waits] + wob_steps() + wprep_steps(0, True))
        toks.clear()
        _run(aproj_steps(CUT, S - CUT))

    pl.run_scoped(phase1, pltpu.VMEM((M, 3 * M), bf16), pltpu.VMEM((LT, M // 2, 128), u32),
                  pltpu.VMEM((LT, H * PITCH, 128), f32), pltpu.VMEM((3 * M // 2, M), u32))

    def phase23(s_v, ctx_v, out_v):
        HB = BQ // 2

        def attn_steps(j):
            orders = '76543210,76543210'.split(',')
            tasks = [(e, int(ch)) for e in range(2) for ch in orders[e]]
            rowmax = {}

            def segments(qi):
                segs, k0 = [], 0
                while k0 < qi * BQ:
                    wd = CW if k0 + CW <= qi * BQ else BQ
                    segs.append((k0, wd))
                    k0 += wd
                return segs

            def p1_steps(n):
                e, qi = tasks[n]
                sb = s_v.at[n % NS]
                r0 = qi * BQ
                state = {"m": None}

                def upd(m, s):
                    for x in _lane_tiles(s):
                        m = x if m is None else jnp.maximum(m, x)
                    return m

                def full(k0, wd):
                    def f():
                        s = lax.dot_general(pin(_ld(q_v.at[e], slice(r0, r0 + BQ))), _ld(k_v.at[e], slice(k0, k0 + wd)), NT,
                                            preferred_element_type=f32)
                        sb[:, k0:k0 + wd] = s
                        state["m"] = upd(state["m"], s)
                    return f

                def diag():
                    neg = NEG * D ** -0.5 * LOG2E
                    if DIAG == 0:
                        tri = (lax.broadcasted_iota(jnp.int32, (BQ, BQ), 1)
                               <= lax.broadcasted_iota(jnp.int32, (BQ, BQ), 0))
                        s = lax.dot_general(_ld(q_v.at[e], slice(r0, r0 + BQ)), _ld(k_v.at[e], slice(r0, r0 + BQ)), NT,
                                            preferred_element_type=f32)
                        s = jnp.where(tri, s, neg)
                        sb[:, r0:r0 + BQ] = s
                        md = upd(None, s)
                    else:
                        tri = (lax.broadcasted_iota(jnp.int32, (HB, HB), 1)
                               <= lax.broadcasted_iota(jnp.int32, (HB, HB), 0))
                        sa = lax.dot_general(_ld(q_v.at[e], slice(r0, r0 + BQ)), _ld(k_v.at[e], slice(r0, r0 + HB)), NT,
                                             preferred_element_type=f32)
                        sa = jnp.concatenate([jnp.where(tri, sa[:HB], neg), sa[HB:]], axis=0)
                        sc = lax.dot_general(_ld(q_v.at[e], slice(r0 + HB, r0 + BQ)), _ld(k_v.at[e], slice(r0 + HB, r0 + BQ)), NT,
                                             preferred_element_type=f32)
                        sc = jnp.where(tri, sc, neg)
                        sb[:, r0:r0 + HB] = sa
                        sb[HB:BQ, r0 + HB:r0 + BQ] = sc
                        md = jnp.concatenate([sa[:HB], jnp.maximum(sa[HB:], sc)], axis=0)
                    m = md if state["m"] is None else jnp.maximum(state["m"], md)
                    rowmax[n] = jnp.max(m, axis=1, keepdims=True)
                return [full(*sg) for sg in segments(qi)] + [diag]

            def p2_steps(n):
                e, qi = tasks[n]
                sb = s_v.at[n % NS]
                r0 = qi * BQ
                state = {"l": None, "acc": None}

                def lsum(l, p):
                    t = None
                    for x in _lane_tiles(p):
                        t = x if t is None else t + x
                    return t if l is None else l + t

                def full(k0, wd):
                    def f():
                        p = jnp.exp2(sb[:, k0:k0 + wd] - rowmax[n])
                        state["l"] = lsum(state["l"], p)
                        o = jnp.dot(p.astype(bf16), _ld(v_v.at[e], slice(k0, k0 + wd)), preferred_element_type=f32)
                        state["acc"] = o if state["acc"] is None else state["acc"] + o
                    return f

                def diag():
                    m = rowmax[n]
                    if DIAG == 0:
                        p = jnp.exp2(sb[:, r0:r0 + BQ] - m)
                        l = lsum(None, p)
                        acc = jnp.dot(p.astype(bf16), _ld(v_v.at[e], slice(r0, r0 + BQ)), preferred_element_type=f32)
                    else:
                        pa = jnp.exp2(sb[:, r0:r0 + HB] - m)
                        pc = jnp.exp2(sb[HB:BQ, r0 + HB:r0 + BQ] - m[HB:])
                        oa = jnp.dot(pa.astype(bf16), _ld(v_v.at[e], slice(r0, r0 + HB)), preferred_element_type=f32)
                        oc = jnp.dot(pc.astype(bf16), _ld(v_v.at[e], slice(r0 + HB, r0 + BQ)), preferred_element_type=f32)
                        l = jnp.concatenate([pa[:HB], pa[HB:] + pc], axis=0)
                        acc = jnp.concatenate([oa[:HB], oa[HB:] + oc], axis=0)
                    if state["l"] is not None:
                        l = l + state["l"]
                        acc = acc + state["acc"]
                    l = jnp.sum(l, axis=1, keepdims=True)
                    inv = pl.reciprocal(l, approx=True)
                    inv = inv * (2.0 - l * inv)
                    _st(ctx_v.at[2 * j + e], slice(r0, r0 + BQ), ALL, (acc * inv).astype(bf16))
                return [full(*sg) for sg in segments(qi)] + [diag]

            sa = [(n, f) for n in range(len(tasks)) for f in p1_steps(n)]
            sb_ = [(n, f) for n in range(len(tasks)) for f in p2_steps(n)]
            end_a = {n: i + 1 for i, (n, _) in enumerate(sa)}
            end_b = {n: i + 1 for i, (n, _) in enumerate(sb_)}
            steps, ia, ib, last = [], 0, 0, "b"
            while ia < len(sa) or ib < len(sb_):
                can_a = ia < len(sa) and (sa[ia][0] < NS or ib >= end_b[sa[ia][0] - NS])
                can_b = ib < len(sb_) and (ia >= min(end_a[sb_[ib][0]] + LAG, len(sa)) or not can_a)
                if can_a and (last == "b" or not can_b):
                    steps.append(sa[ia][1])
                    ia, last = ia + 1, "a"
                else:
                    assert ia >= end_a[sb_[ib][0]]
                    steps.append(sb_[ib][1])
                    ib, last = ib + 1, "b"
            n_hi = max(n for n, (e, qi) in enumerate(tasks) if qi * BQ >= CUT)
            cut = steps.index(sb_[end_b[n_hi] - 1][1]) + 1
            return steps[:cut], steps[cut:]

        def pair(j, last):
            if CUT > 0:
                _run(aproj_steps(0, CUT), local_steps(pl.multiple_of(j * RL, RL), LS))
                toks.clear()
            head, tail = attn_steps(j)
            _run(head)
            if last:
                _run(tail, local_steps(j * RL + LS, RL - LS))
            else:
                _run(tail, wprep_steps(j + 1) + aproj_steps(CUT, S - CUT),
                     local_steps(pl.multiple_of(j * RL + LS, RI), RL - LS))
            toks.clear()

        def pair_body(j, c):
            pair(j, False)
            return c

        lax.fori_loop(0, NP - 1, pair_body, 0)
        pair(NP - 1, True)

        gw_cp.wait()
        wo_cp.wait()
        gw = gw_v[...].astype(f32).reshape(1, M)
        blocks = [tuple(int(v) for v in b.split(':')) for b in '0:2048:0:512,0:2048:512:384,0:1024:896:128,1024:1024:896:128'.split(',')]

        def out_copy(i):
            r, nr, c, nc = blocks[i]
            return pltpu.make_async_copy(out_v.at[i % 2, 0:nr, 0:nc], out_hbm.at[r:r + nr, c:c + nc], osem.at[i % 2])

        g = jax.nn.sigmoid(jnp.sum(_ld(x_v, slice(0, S)).astype(f32) * gw, axis=1, keepdims=True))
        for i, (r, nr, c, nc) in enumerate(blocks):
            rows, cols = slice(r, r + nr), slice(c, c + nc)
            a = None
            for h in range(H):
                t = jnp.dot(_ld(ctx_v.at[h], rows), _ld(wo_v, slice(h * D, (h + 1) * D), cols),
                            preferred_element_type=f32)
                a = t if a is None else a + t
            b = jnp.dot(_ld(ob_v, rows), _ld(wobp_v, slice(0, M), cols), preferred_element_type=f32)
            if i >= 2:
                out_copy(i - 2).wait()
            gr = g[r:r + nr]
            out_v[i % 2, 0:nr, 0:nc] = (gr * a + (1.0 - gr) * b).astype(bf16)
            out_copy(i).start()
        out_copy(len(blocks) - 2).wait()
        out_copy(len(blocks) - 1).wait()

    pl.run_scoped(phase23, pltpu.VMEM((NS, BQ, S), f32), pltpu.VMEM((H, S // 2, D), u32), pltpu.VMEM((2, S, 512), bf16))


@jax.jit
def pallas_gated_mix__compressed_kv_cla__sliding_local_dilated__prompt_kernel(
    A_x, A_c_kv, A_w_q, A_w_uk, A_w_uv, A_w_o, B_x, B_wqkv, B_wo, gate_w,
):
    del B_x
    any_spec = pl.BlockSpec(memory_space=pl.ANY)
    out = pl.pallas_call(
        _kernel,
        out_shape=jax.ShapeDtypeStruct((S, M), bf16),
        in_specs=[any_spec] * 9,
        out_specs=any_spec,
        scratch_shapes=[
            pltpu.VMEM((S // 2, M), u32), pltpu.VMEM((S // 2, DC), u32),
            pltpu.VMEM((M // 8, 8 * WP, D), u32), pltpu.VMEM((DC // 8, 8 * WP, D), u32),
            pltpu.VMEM((DC // 8, 8 * WP, D), u32),
            pltpu.VMEM((H * D // 2, M), u32), pltpu.VMEM((M,), bf16), pltpu.VMEM((M // 2, M), u32),
            pltpu.VMEM((S // 2, M), u32),
            pltpu.VMEM((LT, S, 128), f32), pltpu.VMEM((LT, S + PAD, 128), f32), pltpu.VMEM((LT, S + PAD, 128), f32),
            pltpu.VMEM((M // 2, 2 * D), u32), pltpu.VMEM((DC // 2, 4 * D), u32),
            pltpu.VMEM((2, S // 2, D), u32), pltpu.VMEM((2, S // 2, D), u32), pltpu.VMEM((2, S // 2, D), u32),
            pltpu.SMEM((1,), jnp.int32), pltpu.SemaphoreType.DMA((S // RB + 10 + M // 128,)), pltpu.SemaphoreType.DMA((2,)),
        ],
        compiler_params=pltpu.CompilerParams(vmem_limit_bytes=126 * 1024 * 1024),
    )(
        A_x.reshape(S, M), A_c_kv.reshape(S, DC), A_w_q.reshape(M // 8, 8, H, D), A_w_uk.reshape(DC // 8, 8, H, D),
        A_w_uv.reshape(DC // 8, 8, H, D), A_w_o.reshape(H * D, M), B_wqkv, B_wo, gate_w,
    )
    return out.reshape(1, S, M)
```

```python
import functools

import jax
import jax.numpy as jnp
from jax import lax
import jax.experimental.pallas as pl
import jax.experimental.pallas.tpu as pltpu

S = 2048
M = 1024
H = 32
D = 128
DC = 512
DH = 32
W = 8
DIL = 2
PAD = 16
PITCH = DH + 1
BQ = 256
NQ = S // BQ
NP = H // 2
RB = 256
NB = 256
RP = 256
RI = 16
RL = S // NP
CW = 256
NS = 2
LAG = 1
WP = H // 2 + 1
CUT = 1792
LS = 112
R0 = 512
KS = 4
ALL = slice(None)
LT = M // 128
LOG2E = 1.4426950408889634
NEG = -1e9
NT = (((1,), (1,)), ((), ()))
f32, bf16, u32 = jnp.float32, jnp.bfloat16, jnp.uint32


def _run(*lists):
    items = []
    for k, l in enumerate(lists):
        items += [((i + 0.5) / len(l), k, f) for i, f in enumerate(l)]
    items.sort(key=lambda t: (t[0], t[1]))
    for _, _, f in items:
        f()


def _unpack(u):
    lo = lax.bitcast_convert_type(u << 16, f32)
    hi = lax.bitcast_convert_type(u & jnp.uint32(0xFFFF0000), f32)
    return lo, hi


def _half(rows):
    if isinstance(rows, slice):
        return slice(rows.start // 2, rows.stop // 2)
    start = rows.start // 2
    return pl.ds(start if isinstance(start, int) else pl.multiple_of(start, 8), rows.size // 2)


def _ld(ref, rows, cols=slice(None)):
    return pltpu.bitcast(ref[_half(rows), cols], bf16)


def _st(ref, rows, cols, val):
    ref[_half(rows), cols] = pltpu.bitcast(val, u32)


def _recip(x):
    r = pl.reciprocal(x, approx=True)
    return r * (2.0 - x * r)


def _lane_tiles(x):
    return [x[:, t * 128:(t + 1) * 128] for t in range(x.shape[1] // 128)]


def _kernel(x_hbm, ckv_hbm, wq_hbm, wuk_hbm, wuv_hbm, wo_hbm, wqkv_hbm, wob_hbm, gw_hbm, out_hbm,
            x_v, ckv_v, wq_v, wuk_v, wuv_v, wo_v, gw_v, wobp_v, ob_v, qb_v, kb_v, vb_v,
            wa_v, wb_v, q_v, k_v, v_v, zero_s, sem, osem):
    zero_s[0] = 0
    toks = []

    def pin(lhs):
        if not toks:
            return lhs
        tok = functools.reduce(lambda a, b: a | b, toks)
        toks.clear()
        never = (lax.broadcasted_iota(jnp.int32, (8, 128), 1) + zero_s[0]) < 0
        head = pltpu.bitcast(lhs[0:16, 0:128], u32)
        head = pltpu.bitcast(jnp.where(never, tok, head), bf16)
        top = head if lhs.shape[1] == 128 else jnp.concatenate([head, lhs[0:16, 128:]], axis=1)
        return jnp.concatenate([top, lhs[16:]], axis=0)

    def cp(src, dst, i):
        return pltpu.make_async_copy(src, dst, sem.at[i])

    NX = S // RB
    HR = RB // 2
    x_cp = [cp(x_hbm.bitcast(u32).at[i * HR:(i + 1) * HR, :], x_v.at[i * HR:(i + 1) * HR, :], i) for i in range(NX)]
    gw_cp = cp(gw_hbm, gw_v, NX + 4)
    ckv_cp = cp(ckv_hbm.bitcast(u32), ckv_v, NX + 5)
    def w_cps(src, dst, i):
        return [cp(src.bitcast(u32).at[:, c], dst.at[:, c * WP:c * WP + NP, :], i) for c in range(8)]
    wq_cp = w_cps(wq_hbm, wq_v, NX + 6)
    wuk_cp = w_cps(wuk_hbm, wuk_v, NX + 7)
    wuv_cp = w_cps(wuv_hbm, wuv_v, NX + 8)
    wo_cp = cp(wo_hbm.bitcast(u32), wo_v, NX + 9)

    def wprep_steps(j, tok=False):
        def one(src, dst, r0, n, c0, c1):
            def f():
                u = [src[g, pl.ds(j, 8, stride=WP), :] for g in range(r0 // 8, (r0 + n) // 8)]
                lo, hi = _unpack(jnp.concatenate(u, axis=0))
                lo, hi = lo.astype(bf16), hi.astype(bf16)
                _st(dst, slice(r0, r0 + n), slice(c0, c0 + D), lo)
                _st(dst, slice(r0, r0 + n), slice(c1, c1 + D), hi)
                if tok:
                    toks.extend(pltpu.bitcast(x[i:i + 16], u32) for x in (lo, hi) for i in range(0, n, 16))
            return f
        n = 256
        return ([one(wq_v, wa_v, r0, n, 0, D) for r0 in range(0, M, n)]
                + [one(wuk_v, wb_v, r0, n, 0, D) for r0 in range(0, DC, n)]
                + [one(wuv_v, wb_v, r0, n, 2 * D, 3 * D) for r0 in range(0, DC, n)])

    def aproj_steps(kv_rows, q_rows):
        def kv_piece(r0):
            def f():
                r = slice(r0, r0 + RP)
                y = jnp.dot(pin(_ld(ckv_v, r)), _ld(wb_v, slice(0, DC)), preferred_element_type=f32).astype(bf16)
                _st(k_v.at[0], r, ALL, y[:, 0 * D:1 * D])
                _st(k_v.at[1], r, ALL, y[:, 1 * D:2 * D])
                _st(v_v.at[0], r, ALL, y[:, 2 * D:3 * D])
                _st(v_v.at[1], r, ALL, y[:, 3 * D:4 * D])
            return f

        def q_piece(r0):
            def f():
                r = slice(r0, r0 + RP)
                y = jnp.dot(pin(_ld(x_v, r)), _ld(wa_v, slice(0, M)), preferred_element_type=f32)
                y = (y * (D ** -0.5 * LOG2E)).astype(bf16)
                _st(q_v.at[0], r, ALL, y[:, :D])
                _st(q_v.at[1], r, ALL, y[:, D:])
            return f
        return [kv_piece(r0) for r0 in range(*kv_rows, RP)] + [q_piece(r0) for r0 in range(*q_rows, RP)]

    def local_steps(r0, rows):
        def block(ib):
            def f():
                r = r0 + ib * RI
                qt = [qb_v[t, pl.ds(r, RI), :] for t in range(LT)]
                pos = r + lax.broadcasted_iota(jnp.int32, (RI, 128), 0)
                logits = []
                for w in range(W):
                    acc = None
                    for t in range(LT):
                        pr = qt[t] * kb_v[t, pl.ds(r + PAD - w * DIL, RI), :]
                        acc = pr if acc is None else acc + pr
                    acc = acc + pltpu.roll(acc, 64, 1)
                    acc = acc + pltpu.roll(acc, 32, 1)
                    if w > 0:
                        acc = jnp.where(pos >= w * DIL, acc, NEG * LOG2E)
                    logits.append(acc)
                m = functools.reduce(jnp.maximum, logits)
                ps = [jnp.exp2(l - m) for l in logits]
                inv = _recip(functools.reduce(lambda a, b: a + b, ps))
                ps = [p * inv for p in ps]
                for t in range(LT):
                    o = None
                    for w in range(W):
                        term = ps[w] * vb_v[t, pl.ds(r + PAD - w * DIL, RI), :]
                        o = term if o is None else o + term
                    ob = o.astype(bf16)
                    _st(ob_v, pl.ds(r, RI), slice(t * 128, (t + 1) * 128), ob)
                    toks.append(pltpu.bitcast(ob[0:16], u32))
            return f
        return [block(ib) for ib in range(rows // RI)]

    def phase1(wqkv_v, wob_v, wt_v, wtp_v):
        def wcols(c0, n, i):
            return cp(wqkv_hbm.at[:, c0:c0 + n], wqkv_v.at[:, c0:c0 + n], i)
        wk_cp = [cp(wqkv_hbm.at[t * 128:(t + 1) * 128, M:2 * M], wqkv_v.at[t * 128:(t + 1) * 128, M:2 * M], NX + 10 + t)
                 for t in range(LT)]
        wqkv_cp = [wcols(0, M, NX), None, wcols(2 * M, M, NX + 2)]
        wob_cp = [cp(wob_hbm.bitcast(u32).at[:, t * 128:(t + 1) * 128], wob_v.at[t], NX + 3) for t in range(LT)]
        third = wob_cp + wq_cp + wuk_cp + wuv_cp + [ckv_cp, wo_cp, gw_cp]
        N0 = R0 // RB
        for c in wk_cp[:1] + x_cp[:N0] + wk_cp[1:] + x_cp[N0:] + [wqkv_cp[2], wqkv_cp[0]]:
            c.start()

        def prep_steps(p):
            def tr(mt):
                def f():
                    if p == 1:
                        wk_cp[mt].wait()
                    blk_t = wqkv_v[mt * 128:(mt + 1) * 128, p * M:(p + 1) * M].astype(f32).T
                    for h in range(H):
                        wt_v[mt, h * PITCH:h * PITCH + DH, :] = blk_t[h * DH:(h + 1) * DH, :]
                return f

            def perm(mt):
                def f():
                    for dh in range(DH):
                        rows = wt_v[mt, pl.ds(dh, H, stride=PITCH), :].astype(bf16)
                        _st(wtp_v, slice(p * M + dh * H, p * M + (dh + 1) * H), slice(mt * 128, (mt + 1) * 128), rows)
                        if p != 1:
                            toks.extend(pltpu.bitcast(rows[i:i + 16], u32) for i in range(0, H, 16))
                return f
            return [g(mt) for mt in range(LT) for g in (tr, perm)]

        def proj_steps(p):
            def piece(i, c0):
                def f():
                    if p == 1 and c0 == 0 and i == N0:
                        for c in x_cp[N0:KS]:
                            c.wait()
                    r0 = i * RB
                    y = lax.dot_general(pin(_ld(x_v, slice(r0, r0 + RB))), _ld(wtp_v, slice(p * M + c0, p * M + c0 + NB)), NT,
                                        preferred_element_type=f32)
                    if p == 0:
                        y = y * (DH ** -0.5 * LOG2E)
                    for t, yt in enumerate(_lane_tiles(y)):
                        if p == 0:
                            qb_v[c0 // 128 + t, r0:r0 + RB, :] = yt
                        elif p == 1:
                            kb_v[c0 // 128 + t, PAD + r0:PAD + r0 + RB, :] = yt
                        else:
                            vb_v[c0 // 128 + t, PAD + r0:PAD + r0 + RB, :] = yt
                return f
            return [piece(i, c0) for i in range(N0 if p == 1 else 0, NX) for c0 in range(0, M, NB)]

        def wob_steps():
            def one(j):
                def f():
                    for t in range(LT):
                        lo, hi = _unpack(wob_v[t, pl.ds(j, H, stride=DH // 2), :])
                        rows = jnp.concatenate([lo, hi], axis=0).astype(bf16)
                        _st(wobp_v, slice(2 * j * H, (2 * j + 2) * H), slice(t * 128, (t + 1) * 128), rows)
                        toks.extend(pltpu.bitcast(rows[i:i + 16], u32) for i in range(0, 2 * H, 16))
                return f
            return [one(j) for j in range(DH // 2)]

        kb_v[:, 0:PAD, :] = jnp.zeros((LT, PAD, 128), f32)
        vb_v[:, 0:PAD, :] = jnp.zeros((LT, PAD, 128), f32)
        pk = prep_steps(1)
        y = None
        pk[0]()
        pk[1]()
        for c in x_cp[:N0]:
            c.wait()
        for mt in range(LT):
            for f in pk[2 * mt + 2:2 * mt + 4]:
                f()
            cols = slice(mt * 128, (mt + 1) * 128)
            t = lax.dot_general(_ld(x_v, slice(0, R0), cols), _ld(wtp_v, slice(M, 2 * M), cols), NT,
                                preferred_element_type=f32)
            y = t if y is None else y + t
        for t, yt in enumerate(_lane_tiles(y)):
            kb_v[t, PAD:PAD + R0, :] = yt
        pj = proj_steps(1)
        pv = prep_steps(2)
        per = M // NB
        pj = [None] * (N0 * per) + pj
        for i in range(N0, NX):
            if i < KS:
                _run(pj[i * per:(i + 1) * per])
            else:
                if i == KS:
                    for c in x_cp[KS:] + [wqkv_cp[2], wqkv_cp[0]]:
                        c.wait()
                    for c in third:
                        c.start()
                n0, n1 = [len(pv) * (ii - KS) // (NX - KS) for ii in (i, i + 1)]
                _run(pj[i * per:(i + 1) * per], pv[n0:n1])
        _run(proj_steps(2), prep_steps(0))

        def waits():
            for c in wob_cp + wq_cp + wuk_cp + wuv_cp + [ckv_cp]:
                c.wait()
        _run(proj_steps(0), [waits] + wob_steps() + wprep_steps(0, True))
        toks.clear()
        _run(aproj_steps((CUT, S), (CUT, S)))

    pl.run_scoped(phase1, pltpu.VMEM((M, 3 * M), bf16), pltpu.VMEM((LT, M // 2, 128), u32),
                  pltpu.VMEM((LT, H * PITCH, 128), f32), pltpu.VMEM((3 * M // 2, M), u32))

    def phase23(s_v, ctx_v, out_v):
        HB = BQ // 2

        def attn_steps(j):
            tasks = [(e, qi) for e in range(2) for qi in range(NQ - 1, -1, -1)]
            rowmax = {}

            def segments(qi):
                segs, k0 = [], 0
                while k0 < qi * BQ:
                    wd = CW if k0 + CW <= qi * BQ else BQ
                    segs.append((k0, wd))
                    k0 += wd
                return segs

            def p1_steps(n):
                e, qi = tasks[n]
                sb = s_v.at[n % NS]
                r0 = qi * BQ
                state = {"m": None}

                def upd(m, s):
                    for x in _lane_tiles(s):
                        m = x if m is None else jnp.maximum(m, x)
                    return m

                def full(k0, wd):
                    def f():
                        s = lax.dot_general(pin(_ld(q_v.at[e], slice(r0, r0 + BQ))), _ld(k_v.at[e], slice(k0, k0 + wd)), NT,
                                            preferred_element_type=f32)
                        sb[:, k0:k0 + wd] = s
                        state["m"] = upd(state["m"], s)
                    return f

                def diag():
                    neg = NEG * LOG2E
                    tri = (lax.broadcasted_iota(jnp.int32, (HB, HB), 1)
                           <= lax.broadcasted_iota(jnp.int32, (HB, HB), 0))
                    sa = lax.dot_general(_ld(q_v.at[e], slice(r0, r0 + BQ)), _ld(k_v.at[e], slice(r0, r0 + HB)), NT,
                                         preferred_element_type=f32)
                    sa = jnp.concatenate([jnp.where(tri, sa[:HB], neg), sa[HB:]], axis=0)
                    sc = lax.dot_general(_ld(q_v.at[e], slice(r0 + HB, r0 + BQ)), _ld(k_v.at[e], slice(r0 + HB, r0 + BQ)), NT,
                                         preferred_element_type=f32)
                    sc = jnp.where(tri, sc, neg)
                    sb[:, r0:r0 + HB] = sa
                    sb[HB:BQ, r0 + HB:r0 + BQ] = sc
                    md = jnp.concatenate([sa[:HB], jnp.maximum(sa[HB:], sc)], axis=0)
                    m = md if state["m"] is None else jnp.maximum(state["m"], md)
                    rowmax[n] = jnp.max(m, axis=1, keepdims=True)
                return [full(*sg) for sg in segments(qi)] + [diag]

            def p2_steps(n):
                e, qi = tasks[n]
                sb = s_v.at[n % NS]
                r0 = qi * BQ
                state = {"l": None, "acc": None}

                def lsum(l, p):
                    t = None
                    for x in _lane_tiles(p):
                        t = x if t is None else t + x
                    return t if l is None else l + t

                def full(k0, wd):
                    def f():
                        p = jnp.exp2(sb[:, k0:k0 + wd] - rowmax[n])
                        state["l"] = lsum(state["l"], p)
                        o = jnp.dot(p.astype(bf16), _ld(v_v.at[e], slice(k0, k0 + wd)), preferred_element_type=f32)
                        state["acc"] = o if state["acc"] is None else state["acc"] + o
                    return f

                def diag():
                    m = rowmax[n]
                    pa = jnp.exp2(sb[:, r0:r0 + HB] - m)
                    pc = jnp.exp2(sb[HB:BQ, r0 + HB:r0 + BQ] - m[HB:])
                    oa = jnp.dot(pa.astype(bf16), _ld(v_v.at[e], slice(r0, r0 + HB)), preferred_element_type=f32)
                    oc = jnp.dot(pc.astype(bf16), _ld(v_v.at[e], slice(r0 + HB, r0 + BQ)), preferred_element_type=f32)
                    l = jnp.concatenate([pa[:HB], pa[HB:] + pc], axis=0)
                    acc = jnp.concatenate([oa[:HB], oa[HB:] + oc], axis=0)
                    if state["l"] is not None:
                        l = l + state["l"]
                        acc = acc + state["acc"]
                    l = jnp.sum(l, axis=1, keepdims=True)
                    inv = _recip(l)
                    _st(ctx_v.at[2 * j + e], slice(r0, r0 + BQ), ALL, (acc * inv).astype(bf16))
                return [full(*sg) for sg in segments(qi)] + [diag]

            sa = [(n, f) for n in range(len(tasks)) for f in p1_steps(n)]
            sb_ = [(n, f) for n in range(len(tasks)) for f in p2_steps(n)]
            end_a = {n: i + 1 for i, (n, _) in enumerate(sa)}
            end_b = {n: i + 1 for i, (n, _) in enumerate(sb_)}
            steps, ia, ib, last = [], 0, 0, "b"
            while ia < len(sa) or ib < len(sb_):
                can_a = ia < len(sa) and (sa[ia][0] < NS or ib >= end_b[sa[ia][0] - NS])
                can_b = ib < len(sb_) and (ia >= min(end_a[sb_[ib][0]] + LAG, len(sa)) or not can_a)
                if can_a and (last == "b" or not can_b):
                    steps.append(sa[ia][1])
                    ia, last = ia + 1, "a"
                else:
                    assert ia >= end_a[sb_[ib][0]]
                    steps.append(sb_[ib][1])
                    ib, last = ib + 1, "b"
            n_hi = max(n for n, (e, qi) in enumerate(tasks) if qi * BQ >= CUT)
            cut = steps.index(sb_[end_b[n_hi] - 1][1]) + 1
            return steps[:cut], steps[cut:]

        def pair(j, last):
            _run(aproj_steps((0, CUT), (0, CUT)), local_steps(pl.multiple_of(j * RL, RL), LS))
            toks.clear()
            head, tail = attn_steps(j)
            _run(head)
            if last:
                _run(tail, local_steps(j * RL + LS, RL - LS))
            else:
                _run(tail, wprep_steps(j + 1) + aproj_steps((CUT, S), (CUT, S)),
                     local_steps(pl.multiple_of(j * RL + LS, RI), RL - LS))
            toks.clear()

        def pair_body(j, c):
            pair(j, False)
            return c

        lax.fori_loop(0, NP - 1, pair_body, 0)
        pair(NP - 1, True)

        gw_cp.wait()
        wo_cp.wait()
        gw = gw_v[...].astype(f32).reshape(1, M)
        blocks = [(0, S, 0, 512), (0, S, 512, 384), (0, S // 2, 896, 128), (S // 2, S // 2, 896, 128)]

        def out_copy(i):
            r, nr, c, nc = blocks[i]
            return pltpu.make_async_copy(out_v.at[i % 2, 0:nr, 0:nc], out_hbm.at[r:r + nr, c:c + nc], osem.at[i % 2])

        g = jax.nn.sigmoid(jnp.sum(_ld(x_v, slice(0, S)).astype(f32) * gw, axis=1, keepdims=True))
        for i, (r, nr, c, nc) in enumerate(blocks):
            rows, cols = slice(r, r + nr), slice(c, c + nc)
            a = None
            for h in range(H):
                t = jnp.dot(_ld(ctx_v.at[h], rows), _ld(wo_v, slice(h * D, (h + 1) * D), cols),
                            preferred_element_type=f32)
                a = t if a is None else a + t
            b = jnp.dot(_ld(ob_v, rows), _ld(wobp_v, slice(0, M), cols), preferred_element_type=f32)
            if i >= 2:
                out_copy(i - 2).wait()
            gr = g[r:r + nr]
            out_v[i % 2, 0:nr, 0:nc] = (gr * a + (1.0 - gr) * b).astype(bf16)
            out_copy(i).start()
        out_copy(len(blocks) - 2).wait()
        out_copy(len(blocks) - 1).wait()

    pl.run_scoped(phase23, pltpu.VMEM((NS, BQ, S), f32), pltpu.VMEM((H, S // 2, D), u32), pltpu.VMEM((2, S, 512), bf16))


@jax.jit
def pallas_gated_mix__compressed_kv_cla__sliding_local_dilated__prompt_kernel(
    A_x, A_c_kv, A_w_q, A_w_uk, A_w_uv, A_w_o, B_x, B_wqkv, B_wo, gate_w,
):
    del B_x
    any_spec = pl.BlockSpec(memory_space=pl.ANY)
    out = pl.pallas_call(
        _kernel,
        out_shape=jax.ShapeDtypeStruct((S, M), bf16),
        in_specs=[any_spec] * 9,
        out_specs=any_spec,
        scratch_shapes=[
            pltpu.VMEM((S // 2, M), u32), pltpu.VMEM((S // 2, DC), u32),
            pltpu.VMEM((M // 8, 8 * WP, D), u32), pltpu.VMEM((DC // 8, 8 * WP, D), u32),
            pltpu.VMEM((DC // 8, 8 * WP, D), u32),
            pltpu.VMEM((H * D // 2, M), u32), pltpu.VMEM((M,), bf16), pltpu.VMEM((M // 2, M), u32),
            pltpu.VMEM((S // 2, M), u32),
            pltpu.VMEM((LT, S, 128), f32), pltpu.VMEM((LT, S + PAD, 128), f32), pltpu.VMEM((LT, S + PAD, 128), f32),
            pltpu.VMEM((M // 2, 2 * D), u32), pltpu.VMEM((DC // 2, 4 * D), u32),
            pltpu.VMEM((2, S // 2, D), u32), pltpu.VMEM((2, S // 2, D), u32), pltpu.VMEM((2, S // 2, D), u32),
            pltpu.SMEM((1,), jnp.int32), pltpu.SemaphoreType.DMA((S // RB + 10 + M // 128,)), pltpu.SemaphoreType.DMA((2,)),
        ],
        compiler_params=pltpu.CompilerParams(vmem_limit_bytes=126 * 1024 * 1024),
    )(
        A_x.reshape(S, M), A_c_kv.reshape(S, DC), A_w_q.reshape(M // 8, 8, H, D), A_w_uk.reshape(DC // 8, 8, H, D),
        A_w_uv.reshape(DC // 8, 8, H, D), A_w_o.reshape(H * D, M), B_wqkv, B_wo, gate_w,
    )
    return out.reshape(1, S, M)
```
